```python
import jax
import jax.numpy as jnp

def _softmax(x, axis=-1):
    return jax.nn.softmax(x, axis=axis)
def _gelu(x):
    return jax.nn.gelu(x, approximate=True)
def _silu(x):
    return jax.nn.silu(x)
def _sigmoid(x):
    return jax.nn.sigmoid(x)
def _layernorm(x, axis=-1, eps=1e-5):
    m = jnp.mean(x, axis=axis, keepdims=True)
    v = jnp.var(x, axis=axis, keepdims=True)
    return (x - m) / jnp.sqrt(v + eps)
def _scatter_add(tgt, idx, src, axis=0):
    return tgt.at[idx].add(src)
def _segment_sum(src, seg, n):
    return jax.ops.segment_sum(src, seg, n)
class _Rng:
    def __init__(self, key):
        self._k = key
    def _next(self):
        self._k, sub = jax.random.split(self._k)
        return sub
    def normal(self, shape):
        return jax.random.normal(self._next(), shape, dtype=jnp.bfloat16)
    def randint(self, lo, hi, shape):
        return jax.random.randint(self._next(), shape, lo, hi, dtype=jnp.int32)
    def uniform(self, shape, lo=0.0, hi=1.0):
        return jax.random.uniform(self._next(), shape, jnp.bfloat16, lo, hi)
    def permutation(self, n):
        return jax.random.permutation(self._next(), n)


kernel_name = 'standalone__gqa_block_cached__near_ridge'

def setup_inputs():
    _rng = _Rng(jax.random.key(int.from_bytes(__import__("os").urandom(4), "little")))
    _w = (lambda a: (lambda t: t.astype(jnp.bfloat16) if jnp.issubdtype(t.dtype, jnp.floating) else t)(jnp.asarray(a)))
    B, Sq, D = 16, 240, 640
    Hq, Hkv, Sk, Dh = 32, 32, 1024, 128
    assert Hq % Hkv == 0, (Hq, Hkv)
    return {
        "x": _w((lambda *s: _rng.normal(s) * 0.05)(B, Sq, D)),
        "k_cache": _w((lambda *s: _rng.normal(s) * 0.05)(B, Hkv, Sk, Dh)),
        "v_cache": _w((lambda *s: _rng.normal(s) * 0.05)(B, Hkv, Sk, Dh)),
        "wq": _w((lambda *s: _rng.normal(s) * 0.05)(D, Hq * Dh) * (D ** -0.5)),
        "wo": _w((lambda *s: _rng.normal(s) * 0.05)(Hq * Dh, D) * ((Hq * Dh) ** -0.5)),
    }

def reference(x, k_cache, v_cache, wq, wo):
    B, Sq, D = x.shape
    Hq, Dh = 32, 128
    Hkv = k_cache.shape[1]
    rep = Hq // Hkv
    q = (lambda x, *d: x.transpose(*d))((x @ wq).reshape(B, Sq, Hq, Dh), 0, 2, 1, 3)
    k = jnp.repeat(k_cache, rep, axis=1)
    v = jnp.repeat(v_cache, rep, axis=1)
    scores = jnp.einsum("bhqd,bhkd->bhqk", q, k) * (Dh ** -0.5)
    p = _softmax(scores, axis=-1)
    o = jnp.einsum("bhqk,bhkd->bhqd", p, v)
    return (lambda x, *d: x.transpose(*d))(o, 0, 2, 1, 3).reshape(B, Sq, Hq * Dh) @ wo
```

```python
import functools
import jax, jax.numpy as jnp
from jax import lax
import jax.experimental.pallas as pl
import jax.experimental.pallas.tpu as pltpu

B, SQ, D = 16, 240, 640
H, SK, DH = 32, 1024, 128
LOG2E = 1.4426950408889634

def _build(G=8, rcp="newton", nround=2, final="plain", op_delay=1, zero="where", lgate=3, lgate_on="l", lgate_w="v", start_pos="after", nobc=True):
    NG = H // G
    NSTEP = B * NG
    GW = G * DH
    c = (DH ** -0.5) * LOG2E
    opq = 4
    NQ = G // opq

    def kernel(x_hbm, k_hbm, v_hbm, wq_hbm, wo_hbm, out_hbm,
               x_v, wq_v, wo_v, kbuf, vbuf, acc, out_v,
               kv_sem, x_sem, w_sem, out_sem):
        def k_copy(s, slot):
            return pltpu.make_async_copy(k_hbm.at[s], kbuf.at[slot], kv_sem.at[0, slot])

        def v_copy(s, slot):
            return pltpu.make_async_copy(v_hbm.at[s], vbuf.at[slot], kv_sem.at[1, slot])

        def x_copy(b):
            return pltpu.make_async_copy(x_hbm.at[b], x_v.at[b], x_sem.at[b])

        def wq_copy(g):
            return pltpu.make_async_copy(wq_hbm.at[:, pl.ds(g * GW, GW)], wq_v.at[:, pl.ds(g * GW, GW)], w_sem.at[0, g])

        def wo_copy(g):
            return pltpu.make_async_copy(wo_hbm.at[pl.ds(g * GW, GW)], wo_v.at[pl.ds(g * GW, GW)], w_sem.at[1, g])

        def out_copy(b):
            return pltpu.make_async_copy(out_v, out_hbm.at[b], out_sem.at[0])

        x_copy(0).start()
        wq_copy(0).start()
        k_copy(0, 0).start()
        v_copy(0, 0).start()
        wo_copy(0).start()

        def step(s, carry):
            b = lax.shift_right_logical(s, NG.bit_length() - 1)
            g = lax.bitwise_and(s, NG - 1)
            slot = lax.bitwise_and(s, 1)

            @pl.when(g == 0)
            def _():
                @pl.when(b + 1 < B)
                def _():
                    x_copy(b + 1).start()
                x_copy(b).wait()

            @pl.when(b == 0)
            def _():
                @pl.when(g + 1 < NG)
                def _():
                    wq_copy(g + 1).start()
                    wo_copy(g + 1).start()
                wq_copy(g).wait()
                wo_copy(g).wait()

            nxt_s = jnp.minimum(s + 1, NSTEP - 1)
            def starts():
                k_copy(nxt_s, 1 - slot).start()
                v_copy(nxt_s, 1 - slot).start()
            if start_pos == "before":
                starts()
            k_copy(s, slot).wait()
            v_copy(s, slot).wait()
            if start_pos == "after":
                starts()

            col = pl.multiple_of(g * GW, GW)
            q = jnp.dot(x_v[b], wq_v[:, pl.ds(col, GW)], preferred_element_type=jnp.float32)
            q = (q * c).astype(jnp.bfloat16)
            if start_pos == "mid":
                starts()

            zs = {}

            def gate_w(w, z):
                if z is None:
                    return w
                u = pltpu.bitcast(w, jnp.uint32)
                u = jnp.concatenate([u[0:8] | z, u[8:]], axis=0)
                return pltpu.bitcast(u, jnp.bfloat16)

            def mkz(l):
                lm = jnp.min(l.reshape(SQ // 8, 8, l.shape[-1]), axis=0)
                return jnp.broadcast_to(lax.shift_right_logical(lax.bitcast_convert_type(lm, jnp.uint32), jnp.uint32(31)), (8, 128))

            def qk(h):
                z = zs.get(h - lgate) if lgate_w == "k" and lgate else None
                return lax.dot_general(q[:, h * DH:(h + 1) * DH], gate_w(kbuf[slot, h], z), (((1,), (1,)), ((), ())),
                                       preferred_element_type=jnp.float32)

            def recip(l):
                if rcp == "exact":
                    return 1.0 / l
                r = pl.reciprocal(l, approx=True)
                return r * (2.0 - l * r)

            def sm_pv(h, sc):
                m = jnp.max(sc, axis=-1, keepdims=True)
                p = jnp.exp2(sc - m)
                tiles = [p[:, j * 128:(j + 1) * 128] for j in range(8)]
                per = 8 // nround
                parts = []
                for r in range(nround):
                    t = tiles[r * per:(r + 1) * per]
                    if per == 4:
                        a = (t[0] + t[1]) + (t[2] + t[3])
                    elif per == 8:
                        a = ((t[0] + t[1]) + (t[2] + t[3])) + ((t[4] + t[5]) + (t[6] + t[7]))
                    parts.append(a)
                    tiles[(r + 1) * per - 1] = jnp.maximum(t[-1], jnp.minimum(a, 0.0))
                pb = jnp.concatenate(tiles, axis=1).astype(jnp.bfloat16)
                z = zs.get(h - lgate) if lgate_w == "v" and lgate else None
                o = jnp.dot(pb, gate_w(vbuf[slot, h], z), preferred_element_type=jnp.float32)
                a = parts[0]
                for x_ in parts[1:]:
                    a = a + x_
                l = jnp.sum(a, axis=-1, keepdims=True)
                r = recip(l)
                on = o * r
                zs[h] = mkz({"l": l, "r": r, "o": on * on}[lgate_on])
                return on.astype(jnp.bfloat16)

            def wo_blk(h0, nh, c0, nc):
                row = pl.multiple_of(col + h0 * DH, DH)
                return wo_v[pl.ds(row, nh * DH), c0 * 128:(c0 + nc) * 128]

            def op(j, y):
                oc = jnp.concatenate(outs[j * opq:(j + 1) * opq], axis=1)
                return y + jnp.dot(oc, wo_blk(j * opq, opq, 0, 5), preferred_element_type=jnp.float32)

            def op_final(j, y):
                h0 = j * opq
                o = outs[h0:h0 + 4]
                if final == "plain":
                    return op(j, y)
                dot = lambda a, w: jnp.dot(a, w, preferred_element_type=jnp.float32)
                if final == "pairs":
                    o01 = jnp.concatenate(o[0:2], axis=1)
                    o23 = jnp.concatenate(o[2:4], axis=1)
                    ya = y[:, 0:256] + dot(o01, wo_blk(h0, 2, 0, 2))
                    yb = y[:, 256:512] + dot(o01, wo_blk(h0, 2, 2, 2))
                    ya = ya + dot(o23, wo_blk(h0 + 2, 2, 0, 2))
                    yb = yb + dot(o23, wo_blk(h0 + 2, 2, 2, 2))
                    yc = y[:, 512:640] + dot(jnp.concatenate(o, axis=1), wo_blk(h0, 4, 4, 1))
                    return jnp.concatenate([ya, yb, yc], axis=1)
                if final == "nsplit":
                    ya = y[:, 0:512]
                    for i in range(4):
                        ya = ya + dot(o[i], wo_blk(h0 + i, 1, 0, 4))
                    yc = y[:, 512:640] + dot(jnp.concatenate(o, axis=1), wo_blk(h0, 4, 4, 1))
                    return jnp.concatenate([ya, yc], axis=1)

            outs = []
            if zero == "where":
                y = jnp.where(g == 0, 0.0, acc[...])
            done = 0
            sc = qk(0)
            for h in range(G):
                nxt = qk(h + 1) if h + 1 < G else None
                if h == G - 1:
                    while done < NQ - 1:
                        y = op(done, y); done += 1
                outs.append(sm_pv(h, sc))
                sc = nxt
                while done < NQ - 2 and (done + 1) * opq - 1 + op_delay <= h:
                    y = op(done, y); done += 1
            y = op_final(NQ - 1, y)
            acc[...] = y

            @pl.when(g == NG - 1)
            def _():
                @pl.when(b > 0)
                def _():
                    out_copy(b - 1).wait()
                out_v[...] = acc[...].astype(out_v.dtype)
                out_copy(b).start()
            return carry

        lax.fori_loop(0, NSTEP, step, 0)
        k_copy(NSTEP - 1, NSTEP % 2).wait()
        v_copy(NSTEP - 1, NSTEP % 2).wait()
        out_copy(B - 1).wait()

    def fn(x, k_cache, v_cache, wq, wo):
        k4 = k_cache.reshape(NSTEP, G, SK, DH)
        v4 = v_cache.reshape(NSTEP, G, SK, DH)
        return pl.pallas_call(
            kernel,
            in_specs=[pl.BlockSpec(memory_space=pl.ANY)] * 5,
            out_specs=pl.BlockSpec(memory_space=pl.ANY),
            out_shape=jax.ShapeDtypeStruct((B, SQ, D), jnp.bfloat16),
            scratch_shapes=[
                pltpu.VMEM((B, SQ, D), jnp.bfloat16),
                pltpu.VMEM((D, H * DH), jnp.bfloat16),
                pltpu.VMEM((H * DH, D), jnp.bfloat16),
                pltpu.VMEM((2, G, SK, DH), jnp.bfloat16),
                pltpu.VMEM((2, G, SK, DH), jnp.bfloat16),
                pltpu.VMEM((SQ, D), jnp.float32),
                pltpu.VMEM((SQ, D), jnp.bfloat16),
                pltpu.SemaphoreType.DMA((2, 2)),
                pltpu.SemaphoreType.DMA((B,)),
                pltpu.SemaphoreType.DMA((2, NG)),
                pltpu.SemaphoreType.DMA((1,)),
            ],
            compiler_params=pltpu.CompilerParams(vmem_limit_bytes=110 * 1024 * 1024, disable_bounds_checks=nobc),
        )(x, k4, v4, wq, wo)
    return fn


_FN = _build(G=8)


@jax.jit
def pallas_standalone__gqa_block_cached__near_ridge_kernel(x, k_cache, v_cache, wq, wo):
    return _FN(x, k_cache, v_cache, wq, wo)
```

```python
import functools
import jax, jax.numpy as jnp
from jax import lax
import jax.experimental.pallas as pl
import jax.experimental.pallas.tpu as pltpu

B, SQ, D = 16, 240, 640
H, SK, DH = 32, 1024, 128
LOG2E = 1.4426950408889634
CH = 4
NC = H // CH
CW = CH * DH


def make_order(with_qp, qpq, opq, op_delay, qp_lead, pen):
    nq = H // opq
    order = []
    qp_done = 0
    op_done = 0

    def need_qp(h):
        nonlocal qp_done
        while with_qp and qp_done < H // qpq and qp_done * qpq <= h:
            order.append(("QP", qp_done)); qp_done += 1

    need_qp(0)
    order.append(("QK", 0))
    for h in range(H):
        if h + 1 < H:
            need_qp(h + 1)
            order.append(("QK", h + 1))
        if h == H - pen:
            while op_done < nq - 1:
                order.append(("OP", op_done)); op_done += 1
        order.append(("PV", h))
        need_qp(min(h + qp_lead, H - 1))
        while op_done < nq - 2 and (op_done + 1) * opq - 1 + op_delay <= h:
            order.append(("OP", op_done)); op_done += 1
    while op_done < nq:
        order.append(("OP", op_done)); op_done += 1
    return order


def _build(NB0=8, prof=False, qpq=8, opq=4, op_delay=2, qp_lead=4, pen=1, lgate=3, sgate="all", only=None):
    c = (DH ** -0.5) * LOG2E

    def kernel(x_hbm, k_hbm, v_hbm, wq_hbm, wo_hbm, out_hbm,
               x_v, wq_v, wo_v, kbuf, vbuf, q_v, out_v,
               kv_sem, x_sem, wq_sem, wo_sem, out_sem):
        def k_copy(b, slot):
            return pltpu.make_async_copy(k_hbm.at[b], kbuf.at[slot], kv_sem.at[0, slot])

        def v_copy(b, slot):
            return pltpu.make_async_copy(v_hbm.at[b], vbuf.at[slot], kv_sem.at[1, slot])

        def x_first():
            return pltpu.make_async_copy(x_hbm.at[pl.ds(0, NB0)], x_v.at[pl.ds(0, NB0)], x_sem.at[0])

        def x_copy(b):
            return pltpu.make_async_copy(x_hbm.at[b], x_v.at[b], x_sem.at[1])

        def wq_copy(j):
            return pltpu.make_async_copy(wq_hbm.at[:, pl.ds(j * CW, CW)], wq_v.at[:, pl.ds(j * CW, CW)], wq_sem.at[j])

        def wo_copy():
            return pltpu.make_async_copy(wo_hbm, wo_v, wo_sem.at[0])

        def out_copy(b, slot):
            return pltpu.make_async_copy(out_v.at[slot], out_hbm.at[b], out_sem.at[slot])

        NGRP = B // NB0
        import contextlib
        scope = (lambda n: jax.named_scope(n)) if prof else (lambda n: contextlib.nullcontext())

        def x_grp(gi):
            return pltpu.make_async_copy(x_hbm.at[pl.ds(gi * NB0, NB0)], x_v.at[pl.ds(gi * NB0, NB0)], x_sem.at[0])

        x_grp(0).start()
        wq_copy(0).start()

        def phase0(gi, j):
            first = gi == 0

            @pl.when(jnp.logical_and(first, j == 0))
            def _():
                for t in range(1, NC):
                    wq_copy(t).start()

            @pl.when(jnp.logical_and(first, j == 1))
            def _():
                k_copy(0, 0).start()
                v_copy(0, 0).start()

            @pl.when(jnp.logical_and(first, j == 4))
            def _():
                wo_copy().start()

            @pl.when(first)
            def _():
                wq_copy(j).wait()

            with scope('p0comp'):
                col = pl.multiple_of(j * CW, CW)
                b0 = pl.multiple_of(gi * NB0, NB0)
                xs = x_v[pl.ds(b0, NB0)].reshape(NB0 * SQ, D)
                q = jnp.dot(xs, wq_v[:, pl.ds(col, CW)], preferred_element_type=jnp.float32)
                q_v[:, pl.ds(col, CW)] = pltpu.bitcast((q * c).astype(jnp.bfloat16), jnp.uint32)

        def block(b, with_qp):
            slot = lax.bitwise_and(b, 1)
            bi = lax.bitwise_and(b, NB0 - 1)
            gnext = b // NB0 + 1

            @pl.when(jnp.logical_and(bi == 1, gnext < NGRP))
            def _():
                x_grp(gnext).start()

            @pl.when(b + 1 < B)
            def _():
                k_copy(b + 1, 1 - slot).start()
                v_copy(b + 1, 1 - slot).start()

            @pl.when(b >= 2)
            def _():
                out_copy(b - 2, slot).wait()

            k_copy(b, slot).wait()
            v_copy(b, slot).wait()

            qs = {}
            zs = {}
            raw = {}
            scs = {}
            outs = {}
            if not with_qp:
                row = pl.multiple_of(bi * (SQ // 2), SQ // 2)
                qall = pltpu.bitcast(q_v[pl.ds(row, SQ // 2), :], jnp.bfloat16)
                for h in range(H):
                    qs[h] = qall[:, h * DH:(h + 1) * DH]

            def gate_w(w, z):
                if z is None:
                    return w
                u = pltpu.bitcast(w, jnp.uint32)
                u = jnp.concatenate([u[0:8] | z, u[8:]], axis=0)
                return pltpu.bitcast(u, jnp.bfloat16)

            def mkz(l):
                lm = jnp.min(l.reshape(SQ // 8, 8, l.shape[-1]), axis=0)
                return jnp.broadcast_to(
                    lax.shift_right_logical(lax.bitcast_convert_type(lm, jnp.uint32), jnp.uint32(31)), (8, 128))

            def qp(j):
                q = jnp.dot(x_v[b], wq_v[:, j * qpq * DH:(j + 1) * qpq * DH], preferred_element_type=jnp.float32)
                q = (q * c).astype(jnp.bfloat16)
                for i in range(qpq):
                    qs[j * qpq + i] = q[:, i * DH:(i + 1) * DH]

            def qk(h):
                scs[h] = lax.dot_general(qs[h], kbuf[slot, h], (((1,), (1,)), ((), ())),
                                         preferred_element_type=jnp.float32)

            def pv(h):
                sc = scs.pop(h)
                if h >= 1 and sgate == "all":
                    s0 = jnp.maximum(sc[:, :128], jnp.minimum(raw[h - 1], -3e38))
                    sc = jnp.concatenate([s0, sc[:, 128:]], axis=1)
                m = jnp.max(sc, axis=-1, keepdims=True)
                p = jnp.exp2(sc - m)
                tiles = [p[:, j * 128:(j + 1) * 128] for j in range(8)]
                parts = []
                for r in range(2):
                    t = tiles[r * 4:(r + 1) * 4]
                    a = (t[0] + t[1]) + (t[2] + t[3])
                    parts.append(a)
                    tiles[r * 4 + 3] = jnp.maximum(t[3], jnp.minimum(a, 0.0))
                pb = jnp.concatenate(tiles, axis=1).astype(jnp.bfloat16)
                z = zs.get(h - lgate) if lgate else None
                o = jnp.dot(pb, gate_w(vbuf[slot, h], z), preferred_element_type=jnp.float32)
                raw[h] = o
                l = jnp.sum(parts[0] + parts[1], axis=-1, keepdims=True)
                r = pl.reciprocal(l, approx=True)
                r = r * (2.0 - l * r)
                zs[h] = mkz(l)
                outs[h] = (o * r).astype(jnp.bfloat16)

            y = None
            for kind, i in make_order(with_qp, qpq, opq, op_delay, qp_lead, pen):
                if kind == "QP":
                    qp(i)
                elif kind == "QK":
                    qk(i)
                elif kind == "PV":
                    pv(i)
                else:
                    oc = jnp.concatenate([outs[i * opq + t] for t in range(opq)], axis=1)
                    d = jnp.dot(oc, wo_v[i * opq * DH:(i + 1) * opq * DH, :], preferred_element_type=jnp.float32)
                    y = d if y is None else y + d
            out_v[slot] = y.astype(out_v.dtype)
            out_copy(b, slot).start()

        def group(gi, carry):
            x_grp(gi).wait()

            def p0(j, cc):
                phase0(gi, j)
                return cc
            lax.fori_loop(0, NC, p0, 0)

            @pl.when(gi == 0)
            def _():
                wo_copy().wait()

            def loop_a(i, cc):
                with scope('blockA'):
                    block(gi * NB0 + i, False)
                return cc
            lax.fori_loop(0, NB0, loop_a, 0)
            return carry

        lax.fori_loop(0, NGRP, group, 0)
        out_copy(B - 2, 0).wait()
        out_copy(B - 1, 1).wait()

    def fn(x, k_cache, v_cache, wq, wo):
        return pl.pallas_call(
            kernel,
            in_specs=[pl.BlockSpec(memory_space=pl.ANY)] * 5,
            out_specs=pl.BlockSpec(memory_space=pl.ANY),
            out_shape=jax.ShapeDtypeStruct((B, SQ, D), jnp.bfloat16),
            scratch_shapes=[
                pltpu.VMEM((B, SQ, D), jnp.bfloat16),
                pltpu.VMEM((D, H * DH), jnp.bfloat16),
                pltpu.VMEM((H * DH, D), jnp.bfloat16),
                pltpu.VMEM((2, H, SK, DH), jnp.bfloat16),
                pltpu.VMEM((2, H, SK, DH), jnp.bfloat16),
                pltpu.VMEM((NB0 * SQ // 2, H * DH), jnp.uint32),
                pltpu.VMEM((2, SQ, D), jnp.bfloat16),
                pltpu.SemaphoreType.DMA((2, 2)),
                pltpu.SemaphoreType.DMA((2,)),
                pltpu.SemaphoreType.DMA((NC,)),
                pltpu.SemaphoreType.DMA((1,)),
                pltpu.SemaphoreType.DMA((2,)),
            ],
            compiler_params=pltpu.CompilerParams(vmem_limit_bytes=120 * 1024 * 1024, disable_bounds_checks=True),
        )(x, k_cache, v_cache, wq, wo)
    return fn


_FN = _build()


@jax.jit
def pallas_standalone__gqa_block_cached__near_ridge_kernel(x, k_cache, v_cache, wq, wo):
    return _FN(x, k_cache, v_cache, wq, wo)
```

```python
import contextlib
import jax, jax.numpy as jnp
from jax import lax
import jax.experimental.pallas as pl
import jax.experimental.pallas.tpu as pltpu

B, SQ, D = 16, 240, 640
H, SK, DH = 32, 1024, 128
LOG2E = 1.4426950408889634
NB0 = 8
NGRP = B // NB0
CH = 4
NC = H // CH
CW = CH * DH
PCH = 2
NP = NC // PCH
PW = PCH * CW
SB = 2


def make_order(opq, op_delay, pen):
    nq = H // opq
    order = [("QK", 0)]
    op_done = 0
    for h in range(H):
        if h + 1 < H:
            order.append(("QK", h + 1))
        if h == H - pen:
            while op_done < nq - 1:
                order.append(("OP", op_done)); op_done += 1
        order.append(("PV", h))
        while op_done < nq - 2 and (op_done + 1) * opq - 1 + op_delay <= h:
            order.append(("OP", op_done)); op_done += 1
    while op_done < nq:
        order.append(("OP", op_done)); op_done += 1
    return order


def _build(prof=False, opq=16, op_delay=2, pen=1, lgate=3, u32kv=False, u32w=False, u32x=False):
    c = (DH ** -0.5) * LOG2E
    scope = (lambda n: jax.named_scope(n)) if prof else (lambda n: contextlib.nullcontext())

    def kernel(x_hbm, k_hbm, v_hbm, wq_hbm, wo_hbm, out_hbm,
               x_v, wq_v, wo_v, kbuf, vbuf, q_v, out_v,
               kv_sem, x_sem, wq_sem, wo_sem, out_sem):
        if u32kv:
            k_hbm = k_hbm.bitcast(jnp.uint32)
            v_hbm = v_hbm.bitcast(jnp.uint32)
        if u32w:
            wq_hbm = wq_hbm.bitcast(jnp.uint32)
            wo_hbm = wo_hbm.bitcast(jnp.uint32)
        if u32x:
            x_hbm = x_hbm.bitcast(jnp.uint32)
        asb = lambda v, f: pltpu.bitcast(v, jnp.bfloat16) if f else v

        def k_copy(b, slot):
            return pltpu.make_async_copy(k_hbm.at[b], kbuf.at[slot], kv_sem.at[0, slot])

        def v_copy(b, slot):
            return pltpu.make_async_copy(v_hbm.at[b], vbuf.at[slot], kv_sem.at[1, slot])

        def x_pair(i):
            return pltpu.make_async_copy(x_hbm.at[pl.ds(i * SB, SB)], x_v.at[pl.ds(i * SB, SB)], x_sem.at[i])

        def x_rest():
            return pltpu.make_async_copy(x_hbm.at[pl.ds(NB0, B - NB0)], x_v.at[pl.ds(NB0, B - NB0)],
                                         x_sem.at[NB0 // SB])

        def wq_copy(j):
            return pltpu.make_async_copy(wq_hbm.at[:, pl.ds(j * CW, CW)], wq_v.at[:, pl.ds(j * CW, CW)], wq_sem.at[j])

        def wo_copy():
            return pltpu.make_async_copy(wo_hbm, wo_v, wo_sem.at[0])

        def out_copy(b, slot):
            return pltpu.make_async_copy(out_v.at[slot], out_hbm.at[b], out_sem.at[slot])

        def qproj(b0, nb, qrow, col, width):
            xs = x_v[pl.ds(b0, nb)]
            xs = asb(xs.reshape(nb * x_v.shape[1], D), u32x)
            q = jnp.dot(xs, asb(wq_v[:, pl.ds(col, width)], u32w), preferred_element_type=jnp.float32)
            q_v[pl.ds(qrow, nb * SQ // 2), pl.ds(col, width)] = pltpu.bitcast((q * c).astype(jnp.bfloat16), jnp.uint32)

        NSP = NB0 // SB
        x_pair(0).start()
        wq_copy(0).start()

        def starter(i, carry):
            p = lax.rem(i, NSP)
            j = lax.div(i, NSP)

            @pl.when(i < NSP)
            def _():
                x_pair(p).wait()

            @pl.when(p == 0)
            def _():
                wq_copy(j).wait()

            @pl.when(i + 1 < NSP)
            def _():
                x_pair(i + 1).start()

            @pl.when(i == NSP - 1)
            def _():
                wq_copy(1).start()

            @pl.when(i == NSP)
            def _():
                for t in range(PCH, 2 * PCH):
                    wq_copy(t).start()

            @pl.when(i == NSP + 1)
            def _():
                for t in range(2 * PCH, NC):
                    wq_copy(t).start()

            with scope('starter'):
                b0 = p * SB
                qproj(b0, SB, pl.multiple_of(b0 * (SQ // 2), SB * SQ // 2), pl.multiple_of(j * CW, CW), CW)
            return carry

        lax.fori_loop(0, PCH * NSP, starter, 0)

        def phase0(gi, j):
            first = gi == 0

            @pl.when(first)
            def _():
                for t in range(PCH):
                    wq_copy(j * PCH + t).wait()

            @pl.when(jnp.logical_and(first, j == 1))
            def _():
                k_copy(0, 0).start()
                v_copy(0, 0).start()

            @pl.when(jnp.logical_and(first, j == 2))
            def _():
                wo_copy().start()

            with scope('p0comp'):
                qproj(pl.multiple_of(gi * NB0, NB0), NB0, 0, pl.multiple_of(j * PW, PW), PW)

        def block(b):
            slot = lax.bitwise_and(b, 1)
            bi = lax.bitwise_and(b, NB0 - 1)

            @pl.when(b == 1)
            def _():
                x_rest().start()

            @pl.when(b + 1 < B)
            def _():
                k_copy(b + 1, 1 - slot).start()
                v_copy(b + 1, 1 - slot).start()

            @pl.when(b >= 2)
            def _():
                out_copy(b - 2, slot).wait()

            k_copy(b, slot).wait()
            v_copy(b, slot).wait()

            zs = {}
            raw = {}
            scs = {}
            outs = {}
            row = pl.multiple_of(bi * (SQ // 2), SQ // 2)
            qall = pltpu.bitcast(q_v[pl.ds(row, SQ // 2), :], jnp.bfloat16)

            def gate_w(w, z):
                if z is None:
                    return asb(w, u32kv)
                u = w if u32kv else pltpu.bitcast(w, jnp.uint32)
                u = jnp.concatenate([u[0:8] | z, u[8:]], axis=0)
                return pltpu.bitcast(u, jnp.bfloat16)

            def mkz(l):
                lm = jnp.min(l.reshape(SQ // 8, 8, l.shape[-1]), axis=0)
                return jnp.broadcast_to(
                    lax.shift_right_logical(lax.bitcast_convert_type(lm, jnp.uint32), jnp.uint32(31)), (8, 128))

            def qk(h):
                scs[h] = lax.dot_general(qall[:, h * DH:(h + 1) * DH], asb(kbuf[slot, h], u32kv), (((1,), (1,)), ((), ())),
                                         preferred_element_type=jnp.float32)

            def pv(h):
                sc = scs.pop(h)
                if h >= 1:
                    s0 = jnp.maximum(sc[:, :128], jnp.minimum(raw[h - 1], -3e38))
                    sc = jnp.concatenate([s0, sc[:, 128:]], axis=1)
                m = jnp.max(sc, axis=-1, keepdims=True)
                p = jnp.exp2(sc - m)
                tiles = [p[:, j * 128:(j + 1) * 128] for j in range(8)]
                parts = []
                for r in range(2):
                    t = tiles[r * 4:(r + 1) * 4]
                    a = (t[0] + t[1]) + (t[2] + t[3])
                    parts.append(a)
                    tiles[r * 4 + 3] = jnp.maximum(t[3], jnp.minimum(a, 0.0))
                pb = jnp.concatenate(tiles, axis=1).astype(jnp.bfloat16)
                z = zs.get(h - lgate) if lgate else None
                o = jnp.dot(pb, gate_w(vbuf[slot, h], z), preferred_element_type=jnp.float32)
                raw[h] = o
                l = jnp.sum(parts[0] + parts[1], axis=-1, keepdims=True)
                r = pl.reciprocal(l, approx=True)
                r = r * (2.0 - l * r)
                zs[h] = mkz(l)
                outs[h] = (o * r).astype(jnp.bfloat16)

            y = None
            for kind, i in make_order(opq, op_delay, pen):
                if kind == "QK":
                    qk(i)
                elif kind == "PV":
                    pv(i)
                else:
                    oc = jnp.concatenate([outs[i * opq + t] for t in range(opq)], axis=1)
                    wr = opq * DH // (2 if u32w else 1)
                    d = jnp.dot(oc, asb(wo_v[i * wr:(i + 1) * wr, :], u32w), preferred_element_type=jnp.float32)
                    y = d if y is None else y + d
            out_v[slot] = y.astype(out_v.dtype)
            out_copy(b, slot).start()

        def group(gi, carry):
            @pl.when(gi > 0)
            def _():
                x_rest().wait()

            def p0(j, cc):
                phase0(gi, j)
                return cc
            lax.fori_loop(jnp.where(gi == 0, 1, 0), NP, p0, 0)

            @pl.when(gi == 0)
            def _():
                wo_copy().wait()

            def loop_a(i, cc):
                with scope('blockA'):
                    block(gi * NB0 + i)
                return cc
            lax.fori_loop(0, NB0, loop_a, 0)
            return carry

        lax.fori_loop(0, NGRP, group, 0)
        out_copy(B - 2, 0).wait()
        out_copy(B - 1, 1).wait()

    def vm(shape, f):
        if f:
            return pltpu.VMEM(shape[:-2] + (shape[-2] // 2, shape[-1]), jnp.uint32)
        return pltpu.VMEM(shape, jnp.bfloat16)

    def fn(x, k_cache, v_cache, wq, wo):
        return pl.pallas_call(
            kernel,
            in_specs=[pl.BlockSpec(memory_space=pl.ANY)] * 5,
            out_specs=pl.BlockSpec(memory_space=pl.ANY),
            out_shape=jax.ShapeDtypeStruct((B, SQ, D), jnp.bfloat16),
            scratch_shapes=[
                vm((B, SQ, D), u32x),
                vm((D, H * DH), u32w),
                vm((H * DH, D), u32w),
                vm((2, H, SK, DH), u32kv),
                vm((2, H, SK, DH), u32kv),
                pltpu.VMEM((NB0 * SQ // 2, H * DH), jnp.uint32),
                pltpu.VMEM((2, SQ, D), jnp.bfloat16),
                pltpu.SemaphoreType.DMA((2, 2)),
                pltpu.SemaphoreType.DMA((NB0 // SB + 1,)),
                pltpu.SemaphoreType.DMA((NC,)),
                pltpu.SemaphoreType.DMA((1,)),
                pltpu.SemaphoreType.DMA((2,)),
            ],
            compiler_params=pltpu.CompilerParams(vmem_limit_bytes=120 * 1024 * 1024, disable_bounds_checks=True),
        )(x, k_cache, v_cache, wq, wo)
    return fn


_FN = _build()


@jax.jit
def pallas_standalone__gqa_block_cached__near_ridge_kernel(x, k_cache, v_cache, wq, wo):
    return _FN(x, k_cache, v_cache, wq, wo)
```

```python
import contextlib
import jax, jax.numpy as jnp
from jax import lax
import jax.experimental.pallas as pl
import jax.experimental.pallas.tpu as pltpu

B, SQ, D = 16, 240, 640
H, SK, DH = 32, 1024, 128
LOG2E = 1.4426950408889634
NB0 = 8
NGRP = B // NB0
CH = 4
NC = H // CH
CW = CH * DH
PCH = 2
NP = NC // PCH
PW = PCH * CW
SB = 2


def make_order(opq, op_delay, pen):
    nq = H // opq
    order = [("QK", 0)]
    op_done = 0
    for h in range(H):
        if h + 1 < H:
            order.append(("QK", h + 1))
        if h == H - pen:
            while op_done < nq - 1:
                order.append(("OP", op_done)); op_done += 1
        order.append(("PV", h))
        while op_done < nq - 2 and (op_done + 1) * opq - 1 + op_delay <= h:
            order.append(("OP", op_done)); op_done += 1
    while op_done < nq:
        order.append(("OP", op_done)); op_done += 1
    return order


def _build(prof=False, opq=16, op_delay=2, pen=1, lgate=3, u32kv=False, u32w=False, u32x=False, gate_on="l", op_pos=None, ogate=0, fgate=False, slast=True, med=False, split=()):
    c = (DH ** -0.5) * LOG2E
    scope = (lambda n: jax.named_scope(n)) if prof else (lambda n: contextlib.nullcontext())

    def kernel(x_hbm, k_hbm, v_hbm, wq_hbm, wo_hbm, out_hbm,
               x_v, wq_v, wo_v, kbuf, vbuf, q_v, out_v,
               kv_sem, x_sem, wq_sem, wo_sem, out_sem):
        if u32kv:
            k_hbm = k_hbm.bitcast(jnp.uint32)
            v_hbm = v_hbm.bitcast(jnp.uint32)
        if u32w:
            wq_hbm = wq_hbm.bitcast(jnp.uint32)
            wo_hbm = wo_hbm.bitcast(jnp.uint32)
        if u32x:
            x_hbm = x_hbm.bitcast(jnp.uint32)
        asb = lambda v, f: pltpu.bitcast(v, jnp.bfloat16) if f else v

        def k_copy(b, slot):
            return pltpu.make_async_copy(k_hbm.at[b], kbuf.at[slot], kv_sem.at[0, slot])

        def v_copy(b, slot):
            return pltpu.make_async_copy(v_hbm.at[b], vbuf.at[slot], kv_sem.at[1, slot])

        def x_pair(i):
            return pltpu.make_async_copy(x_hbm.at[pl.ds(i * SB, SB)], x_v.at[pl.ds(i * SB, SB)], x_sem.at[i])

        def x_rest():
            return pltpu.make_async_copy(x_hbm.at[pl.ds(NB0, B - NB0)], x_v.at[pl.ds(NB0, B - NB0)],
                                         x_sem.at[NB0 // SB])

        def wq_copy(j):
            return pltpu.make_async_copy(wq_hbm.at[:, pl.ds(j * CW, CW)], wq_v.at[:, pl.ds(j * CW, CW)], wq_sem.at[j])

        def wo_copy():
            return pltpu.make_async_copy(wo_hbm, wo_v, wo_sem.at[0])

        def out_copy(b, slot):
            return pltpu.make_async_copy(out_v.at[slot], out_hbm.at[b], out_sem.at[slot])

        def qproj(b0, nb, qrow, col, width):
            xs = x_v[pl.ds(b0, nb)]
            xs = asb(xs.reshape(nb * x_v.shape[1], D), u32x)
            q = jnp.dot(xs, asb(wq_v[:, pl.ds(col, width)], u32w), preferred_element_type=jnp.float32)
            q_v[pl.ds(qrow, nb * SQ // 2), pl.ds(col, width)] = pltpu.bitcast((q * c).astype(jnp.bfloat16), jnp.uint32)

        NSP = NB0 // SB
        x_pair(0).start()
        wq_copy(0).start()

        def starter(i, carry):
            p = lax.rem(i, NSP)
            j = lax.div(i, NSP)

            @pl.when(i < NSP)
            def _():
                x_pair(p).wait()

            @pl.when(p == 0)
            def _():
                wq_copy(j).wait()

            @pl.when(i + 1 < NSP)
            def _():
                x_pair(i + 1).start()

            @pl.when(i == NSP - 1)
            def _():
                wq_copy(1).start()

            @pl.when(i == NSP)
            def _():
                for t in range(PCH, 2 * PCH):
                    wq_copy(t).start()

            @pl.when(i == NSP + 1)
            def _():
                for t in range(2 * PCH, NC):
                    wq_copy(t).start()

            with scope('starter'):
                b0 = p * SB
                qproj(b0, SB, pl.multiple_of(b0 * (SQ // 2), SB * SQ // 2), pl.multiple_of(j * CW, CW), CW)
            return carry

        def starter2(i, carry):
            x_pair(i).wait()

            @pl.when(i == 0)
            def _():
                wq_copy(0).wait()
                x_pair(1).start()

            @pl.when(i == 1)
            def _():
                wq_copy(1).start()

            with scope('starter'):
                b0 = i * SB
                qproj(b0, SB, pl.multiple_of(b0 * (SQ // 2), SB * SQ // 2), 0, CW)
            return carry

        def medium(i, carry):
            @pl.when(i == 0)
            def _():
                wq_copy(1).wait()
                x_pair(2).start()
                x_pair(3).start()

            @pl.when(i == 1)
            def _():
                x_pair(2).wait()
                x_pair(3).wait()
                for t in range(PCH, NC):
                    wq_copy(t).start()

            with scope('medium'):
                hb = jnp.minimum(i, 1)
                j = lax.bitwise_and(i + 1, 1)
                b0 = hb * (2 * SB)
                qproj(b0, 2 * SB, pl.multiple_of(b0 * (SQ // 2), SB * SQ), pl.multiple_of(j * CW, CW), CW)
            return carry

        if med:
            lax.fori_loop(0, 2, starter2, 0)
            lax.fori_loop(0, 3, medium, 0)
        else:
            lax.fori_loop(0, PCH * NSP, starter, 0)

        def phase0(gi, j):
            first = gi == 0

            @pl.when(first)
            def _():
                for t in range(PCH):
                    wq_copy(j * PCH + t).wait()

            @pl.when(jnp.logical_and(first, j == 1))
            def _():
                k_copy(0, 0).start()
                v_copy(0, 0).start()

            @pl.when(jnp.logical_and(first, j == 2))
            def _():
                wo_copy().start()

            with scope('p0comp'):
                qproj(pl.multiple_of(gi * NB0, NB0), NB0, 0, pl.multiple_of(j * PW, PW), PW)

        def block(b):
            slot = lax.bitwise_and(b, 1)
            bi = lax.bitwise_and(b, NB0 - 1)

            @pl.when(b == 1)
            def _():
                x_rest().start()

            @pl.when(b + 1 < B)
            def _():
                k_copy(b + 1, 1 - slot).start()
                v_copy(b + 1, 1 - slot).start()

            @pl.when(b >= 2)
            def _():
                out_copy(b - 2, slot).wait()

            k_copy(b, slot).wait()
            v_copy(b, slot).wait()

            zs = {}
            raw = {}
            scs = {}
            outs = {}
            row = pl.multiple_of(bi * (SQ // 2), SQ // 2)
            qall = pltpu.bitcast(q_v[pl.ds(row, SQ // 2), :], jnp.bfloat16)

            def gate_w(w, z):
                if z is None:
                    return asb(w, u32kv)
                u = w if u32kv else pltpu.bitcast(w, jnp.uint32)
                u = jnp.concatenate([u[0:8] | z, u[8:]], axis=0)
                return pltpu.bitcast(u, jnp.bfloat16)

            def mkz(l):
                lm = jnp.min(l.reshape(SQ // 8, 8, l.shape[-1]), axis=0)
                return jnp.broadcast_to(
                    lax.shift_right_logical(lax.bitcast_convert_type(lm, jnp.uint32), jnp.uint32(31)), (8, 128))

            def qk(h):
                scs[h] = lax.dot_general(qall[:, h * DH:(h + 1) * DH], asb(kbuf[slot, h], u32kv), (((1,), (1,)), ((), ())),
                                         preferred_element_type=jnp.float32)

            def pv(h):
                sc = scs.pop(h)
                if h >= 1 and (slast or h < H - 1):
                    s0 = jnp.maximum(sc[:, :128], jnp.minimum(raw[h - 1], -3e38))
                    sc = jnp.concatenate([s0, sc[:, 128:]], axis=1)
                m = jnp.max(sc, axis=-1, keepdims=True)
                p = jnp.exp2(sc - m)
                tiles = [p[:, j * 128:(j + 1) * 128] for j in range(8)]
                parts = []
                for r in range(2):
                    t = tiles[r * 4:(r + 1) * 4]
                    a = (t[0] + t[1]) + (t[2] + t[3])
                    parts.append(a)
                    tiles[r * 4 + 3] = jnp.maximum(t[3], jnp.minimum(a, 0.0))
                pb = jnp.concatenate(tiles, axis=1).astype(jnp.bfloat16)
                z = zs.get(h - lgate) if lgate else None
                vv = gate_w(vbuf[slot, h], z)
                if h in split:
                    o1 = jnp.dot(pb[:, :SK // 2], vv[:SK // 2], preferred_element_type=jnp.float32)
                    o = o1 + jnp.dot(pb[:, SK // 2:], vv[SK // 2:], preferred_element_type=jnp.float32)
                    raw[h] = o1
                else:
                    o = jnp.dot(pb, vv, preferred_element_type=jnp.float32)
                    raw[h] = o
                l = jnp.sum(parts[0] + parts[1], axis=-1, keepdims=True)
                r = pl.reciprocal(l, approx=True)
                r = r * (2.0 - l * r)
                outs[h] = (o * r).astype(jnp.bfloat16)
                z = mkz(l if gate_on == "l" else r)
                if h < ogate:
                    u = pltpu.bitcast(outs[h], jnp.uint32).reshape(SQ // 16, 8, DH)
                    t = [u[i] for i in range(SQ // 16)]
                    while len(t) > 1:
                        t = [t[i] | t[i + 1] for i in range(0, len(t) - 1, 2)] + ([t[-1]] if len(t) % 2 else [])
                    z = z & t[0]
                zs[h] = z

            y = None
            if op_pos is None:
                order = [(k, (i * opq, (i + 1) * opq) if k == "OP" else i) for k, i in make_order(opq, op_delay, pen)]
            else:
                chunks = []
                prev = 0
                for t in op_pos.split(";"):
                    e, p_ = t.split("@")
                    chunks.append((prev, int(e), int(p_))); prev = int(e)
                order = [("QK", 0)]
                for h in range(H):
                    if h + 1 < H:
                        order.append(("QK", h + 1))
                    order.append(("PV", h))
                    for (a0, a1, p_) in chunks:
                        if p_ == h:
                            order.append(("OP", (a0, a1)))
            for kind, i in order:
                if kind == "QK":
                    qk(i)
                elif kind == "PV":
                    pv(i)
                else:
                    a0, a1 = i
                    oc = jnp.concatenate([outs[t] for t in range(a0, a1)], axis=1)
                    f = DH // (2 if u32w else 1)
                    d = jnp.dot(oc, asb(wo_v[a0 * f:a1 * f, :], u32w), preferred_element_type=jnp.float32)
                    if fgate and a1 < H and (H - 1) not in raw and (H - 2) in raw:
                        hh = H - 1 - lgate
                        zs[hh] = zs[hh] & lax.bitcast_convert_type(d[0:8, 0:128], jnp.uint32)
                    y = d if y is None else y + d
            out_v[slot] = y.astype(out_v.dtype)
            out_copy(b, slot).start()

        def group(gi, carry):
            @pl.when(gi > 0)
            def _():
                x_rest().wait()

            def p0(j, cc):
                phase0(gi, j)
                return cc
            lax.fori_loop(jnp.where(gi == 0, 1, 0), NP, p0, 0)

            @pl.when(gi == 0)
            def _():
                wo_copy().wait()

            def loop_a(i, cc):
                with scope('blockA'):
                    block(gi * NB0 + i)
                return cc
            lax.fori_loop(0, NB0, loop_a, 0)
            return carry

        lax.fori_loop(0, NGRP, group, 0)
        out_copy(B - 2, 0).wait()
        out_copy(B - 1, 1).wait()

    def vm(shape, f):
        if f:
            return pltpu.VMEM(shape[:-2] + (shape[-2] // 2, shape[-1]), jnp.uint32)
        return pltpu.VMEM(shape, jnp.bfloat16)

    def fn(x, k_cache, v_cache, wq, wo):
        return pl.pallas_call(
            kernel,
            in_specs=[pl.BlockSpec(memory_space=pl.ANY)] * 5,
            out_specs=pl.BlockSpec(memory_space=pl.ANY),
            out_shape=jax.ShapeDtypeStruct((B, SQ, D), jnp.bfloat16),
            scratch_shapes=[
                vm((B, SQ, D), u32x),
                vm((D, H * DH), u32w),
                vm((H * DH, D), u32w),
                vm((2, H, SK, DH), u32kv),
                vm((2, H, SK, DH), u32kv),
                pltpu.VMEM((NB0 * SQ // 2, H * DH), jnp.uint32),
                pltpu.VMEM((2, SQ, D), jnp.bfloat16),
                pltpu.SemaphoreType.DMA((2, 2)),
                pltpu.SemaphoreType.DMA((NB0 // SB + 1,)),
                pltpu.SemaphoreType.DMA((NC,)),
                pltpu.SemaphoreType.DMA((1,)),
                pltpu.SemaphoreType.DMA((2,)),
            ],
            compiler_params=pltpu.CompilerParams(vmem_limit_bytes=120 * 1024 * 1024, disable_bounds_checks=True),
        )(x, k_cache, v_cache, wq, wo)
    return fn


_FN = _build(op_pos="24@26;28@30;32@31", lgate=4)


@jax.jit
def pallas_standalone__gqa_block_cached__near_ridge_kernel(x, k_cache, v_cache, wq, wo):
    return _FN(x, k_cache, v_cache, wq, wo)
```

```python
import contextlib

import jax
import jax.numpy as jnp
from jax import lax
import jax.experimental.pallas as pl
import jax.experimental.pallas.tpu as pltpu

B, SQ, D = 16, 240, 640
H, SK, DH = 32, 1024, 128
LOG2E = 1.4426950408889634
NB0 = 8
NGRP = B // NB0
CH = 4
CW = CH * DH
PCH = 2
PW = PCH * CW
NP = H * DH // PW
SB = 2
NSP = NB0 // SB
HALF = SQ // 2
LGATE = 3
FILL = 4
SFILL = 3


def _build(prof=False):
    qscale = (DH ** -0.5) * LOG2E
    scope = (lambda n: jax.named_scope(n)) if prof else (lambda n: contextlib.nullcontext())

    def kernel(x_hbm, k_hbm, v_hbm, wq_hbm, wo_hbm, out_hbm,
               x_v, wq_v, wo_v, kbuf, vbuf, q_v, out_v,
               kv_sem, x_sem, wq_sem, wo_sem, out_sem):
        def k_copy(b, slot):
            return pltpu.make_async_copy(k_hbm.at[b], kbuf.at[slot], kv_sem.at[0, slot])

        def v_copy(b, slot):
            return pltpu.make_async_copy(v_hbm.at[b], vbuf.at[slot], kv_sem.at[1, slot])

        def x_pair(i):
            return pltpu.make_async_copy(x_hbm.at[pl.ds(i * SB, SB)], x_v.at[pl.ds(i * SB, SB)], x_sem.at[i])

        def x_rest():
            return pltpu.make_async_copy(x_hbm.at[pl.ds(NB0, B - NB0)], x_v.at[pl.ds(NB0, B - NB0)], x_sem.at[NSP])

        def wq_copy(j):
            return pltpu.make_async_copy(wq_hbm.at[:, pl.ds(j * CW, CW)], wq_v.at[:, pl.ds(j * CW, CW)], wq_sem.at[j])

        def wq_rest():
            return pltpu.make_async_copy(wq_hbm.at[:, pl.ds(PW, H * DH - PW)], wq_v.at[:, pl.ds(PW, H * DH - PW)],
                                         wq_sem.at[PCH])

        def wo_copy():
            return pltpu.make_async_copy(wo_hbm, wo_v, wo_sem.at[0])

        def out_copy(b, slot):
            return pltpu.make_async_copy(out_v.at[slot], out_hbm.at[b], out_sem.at[slot])

        def qproj(b0, nb, qrow, col, width):
            xs = x_v[pl.ds(b0, nb)].reshape(nb * SQ, D)
            q = jnp.dot(xs, wq_v[:, pl.ds(col, width)], preferred_element_type=jnp.float32)
            q_v[pl.ds(qrow, nb * HALF), pl.ds(col, width)] = pltpu.bitcast((q * qscale).astype(jnp.bfloat16), jnp.uint32)

        x_pair(0).start()
        wq_copy(0).start()

        def starter(i, carry):
            p = lax.bitwise_and(i, NSP - 1)
            j = lax.shift_right_logical(i, NSP.bit_length() - 1)

            @pl.when(i < NSP)
            def _():
                x_pair(p).wait()

            @pl.when(p == 0)
            def _():
                wq_copy(j).wait()

            @pl.when(i + 1 < NSP)
            def _():
                x_pair(i + 1).start()

            @pl.when(i == NSP - 1)
            def _():
                wq_copy(1).start()

            @pl.when(i == NSP)
            def _():
                wq_rest().start()

            with scope('starter'):
                qproj(p * SB, SB, pl.multiple_of(p * (SB * HALF), SB * HALF), pl.multiple_of(j * CW, CW), CW)
            return carry

        lax.fori_loop(0, PCH * NSP, starter, 0)

        def qblock(gi, j):
            first = gi == 0

            @pl.when(jnp.logical_and(first, j == 1))
            def _():
                wq_rest().wait()
                k_copy(0, 0).start()
                v_copy(0, 0).start()

            @pl.when(jnp.logical_and(first, j == 2))
            def _():
                wo_copy().start()

            with scope('qblock'):
                qproj(pl.multiple_of(gi * NB0, NB0), NB0, 0, pl.multiple_of(j * PW, PW), PW)

        def attention(b):
            slot = lax.bitwise_and(b, 1)
            bi = lax.bitwise_and(b, NB0 - 1)

            @pl.when(b == 1)
            def _():
                x_rest().start()

            @pl.when(b + 1 < B)
            def _():
                k_copy(b + 1, 1 - slot).start()
                v_copy(b + 1, 1 - slot).start()

            @pl.when(b >= 2)
            def _():
                out_copy(b - 2, slot).wait()

            k_copy(b, slot).wait()
            v_copy(b, slot).wait()

            qall = pltpu.bitcast(q_v[pl.ds(pl.multiple_of(bi * HALF, HALF), HALF), :], jnp.bfloat16)
            scores, release, vgate, outs = {}, {}, {}, {}

            def qk(h):
                scores[h] = lax.dot_general(qall[:, h * DH:(h + 1) * DH], kbuf[slot, h], (((1,), (1,)), ((), ())),
                                            preferred_element_type=jnp.float32)

            def pv(h):
                sc = scores.pop(h)
                if h >= 1:
                    s0 = jnp.maximum(sc[:, :128], jnp.minimum(release[h - 1], -3e38))
                    sc = jnp.concatenate([s0, sc[:, 128:]], axis=1)
                m = jnp.max(sc, axis=-1, keepdims=True)
                p = jnp.exp2(sc - m)
                tiles = [p[:, j * 128:(j + 1) * 128] for j in range(SK // 128)]
                parts = []
                for r in range(2):
                    t = tiles[r * 4:(r + 1) * 4]
                    a = (t[0] + t[1]) + (t[2] + t[3])
                    parts.append(a)
                    tiles[r * 4 + 3] = jnp.maximum(t[3], jnp.minimum(a, 0.0))
                pb = jnp.concatenate(tiles, axis=1).astype(jnp.bfloat16)
                v = vbuf[slot, h]
                if h - LGATE in vgate:
                    u = pltpu.bitcast(v, jnp.uint32)
                    u = jnp.concatenate([u[0:8] | vgate[h - LGATE], u[8:]], axis=0)
                    v = pltpu.bitcast(u, jnp.bfloat16)
                o = jnp.dot(pb, v, preferred_element_type=jnp.float32)
                release[h] = o
                l = jnp.sum(parts[0] + parts[1], axis=-1, keepdims=True)
                r = pl.reciprocal(l, approx=True)
                r = r * (2.0 - l * r)
                outs[h] = o * r
                lm = jnp.min(l.reshape(SQ // 8, 8, 1), axis=0)
                vgate[h] = jnp.broadcast_to(
                    lax.shift_right_logical(lax.bitcast_convert_type(lm, jnp.uint32), jnp.uint32(31)), (8, 128))

            def oproj(h0, h1):
                oc = jnp.concatenate([outs[t] for t in range(h0, h1)], axis=1).astype(jnp.bfloat16)
                return jnp.dot(oc, wo_v[h0 * DH:h1 * DH, :], preferred_element_type=jnp.float32)

            qk(0)
            for h in range(H - 1):
                qk(h + 1)
                pv(h)
            y = oproj(0, FILL)
            release[H - 2] = y[:, SFILL * 128:(SFILL + 1) * 128]
            pv(H - 1)
            y = y + oproj(FILL, H)
            out_v[slot] = y.astype(out_v.dtype)
            out_copy(b, slot).start()

        def group(gi, carry):
            @pl.when(gi > 0)
            def _():
                x_rest().wait()

            def qloop(j, c):
                qblock(gi, j)
                return c
            lax.fori_loop(jnp.where(gi == 0, 1, 0), NP, qloop, 0)

            @pl.when(gi == 0)
            def _():
                wo_copy().wait()

            def aloop(i, c):
                with scope('attention'):
                    attention(gi * NB0 + i)
                return c
            lax.fori_loop(0, NB0, aloop, 0)
            return carry

        lax.fori_loop(0, NGRP, group, 0)
        out_copy(B - 2, 0).wait()
        out_copy(B - 1, 1).wait()

    def fn(x, k_cache, v_cache, wq, wo):
        return pl.pallas_call(
            kernel,
            in_specs=[pl.BlockSpec(memory_space=pl.ANY)] * 5,
            out_specs=pl.BlockSpec(memory_space=pl.ANY),
            out_shape=jax.ShapeDtypeStruct((B, SQ, D), jnp.bfloat16),
            scratch_shapes=[
                pltpu.VMEM((B, SQ, D), jnp.bfloat16),
                pltpu.VMEM((D, H * DH), jnp.bfloat16),
                pltpu.VMEM((H * DH, D), jnp.bfloat16),
                pltpu.VMEM((2, H, SK, DH), jnp.bfloat16),
                pltpu.VMEM((2, H, SK, DH), jnp.bfloat16),
                pltpu.VMEM((NB0 * HALF, H * DH), jnp.uint32),
                pltpu.VMEM((2, SQ, D), jnp.bfloat16),
                pltpu.SemaphoreType.DMA((2, 2)),
                pltpu.SemaphoreType.DMA((NSP + 1,)),
                pltpu.SemaphoreType.DMA((PCH + 1,)),
                pltpu.SemaphoreType.DMA((1,)),
                pltpu.SemaphoreType.DMA((2,)),
            ],
            compiler_params=pltpu.CompilerParams(vmem_limit_bytes=120 * 1024 * 1024, disable_bounds_checks=True),
        )(x, k_cache, v_cache, wq, wo)
    return fn


_FN = _build()


@jax.jit
def pallas_standalone__gqa_block_cached__near_ridge_kernel(x, k_cache, v_cache, wq, wo):
    return _FN(x, k_cache, v_cache, wq, wo)
```

```python
import contextlib

import jax
import jax.numpy as jnp
from jax import lax
import jax.experimental.pallas as pl
import jax.experimental.pallas.tpu as pltpu

B, SQ, D = 16, 240, 640
H, SK, DH = 32, 1024, 128
LOG2E = 1.4426950408889634
NB0 = 8
NGRP = B // NB0
CH = 4
CW = CH * DH
PCH = 2
PW = PCH * CW
NP = H * DH // PW
SB = 2
NSP = NB0 // SB
HALF = SQ // 2
LGATE = 3
FILL = 16
REL_TILES = (1, 2, 3)
OUT_CUTS = (0, 512, D)


def _build(prof=False):
    qscale = (DH ** -0.5) * LOG2E
    scope = (lambda n: jax.named_scope(n)) if prof else (lambda n: contextlib.nullcontext())

    def kernel(x_hbm, k_hbm, v_hbm, wq_hbm, wo_hbm, out_hbm,
               x_v, wq_v, wo_v, kbuf, vbuf, q_v, out_v,
               kv_sem, x_sem, wq_sem, wo_sem, out_sem):
        def k_copy(b, slot):
            return pltpu.make_async_copy(k_hbm.at[b], kbuf.at[slot], kv_sem.at[0, slot])

        def v_copy(b, slot):
            return pltpu.make_async_copy(v_hbm.at[b], vbuf.at[slot], kv_sem.at[1, slot])

        def x_pair(i):
            return pltpu.make_async_copy(x_hbm.at[pl.ds(i * SB, SB)], x_v.at[pl.ds(i * SB, SB)], x_sem.at[i])

        def x_rest():
            return pltpu.make_async_copy(x_hbm.at[pl.ds(NB0, B - NB0)], x_v.at[pl.ds(NB0, B - NB0)], x_sem.at[NSP])

        def wq_copy(j):
            return pltpu.make_async_copy(wq_hbm.at[:, pl.ds(j * CW, CW)], wq_v.at[:, pl.ds(j * CW, CW)], wq_sem.at[j])

        def wq_rest():
            return pltpu.make_async_copy(wq_hbm.at[:, pl.ds(PW, H * DH - PW)], wq_v.at[:, pl.ds(PW, H * DH - PW)],
                                         wq_sem.at[PCH])

        def wo_copy():
            return pltpu.make_async_copy(wo_hbm, wo_v, wo_sem.at[0])

        def out_copies(b, slot):
            return [pltpu.make_async_copy(out_v.at[slot, :, pl.ds(c0, c1 - c0)], out_hbm.at[b, :, pl.ds(c0, c1 - c0)],
                                          out_sem.at[slot, i])
                    for i, (c0, c1) in enumerate(zip(OUT_CUTS[:-1], OUT_CUTS[1:]))]

        def qproj(b0, nb, qrow, col, width):
            xs = x_v[pl.ds(b0, nb)].reshape(nb * SQ, D)
            q = jnp.dot(xs, wq_v[:, pl.ds(col, width)], preferred_element_type=jnp.float32)
            q_v[pl.ds(qrow, nb * HALF), pl.ds(col, width)] = pltpu.bitcast((q * qscale).astype(jnp.bfloat16), jnp.uint32)

        x_pair(0).start()
        wq_copy(0).start()

        def starter(i, carry):
            p = lax.bitwise_and(i, NSP - 1)
            j = lax.shift_right_logical(i, NSP.bit_length() - 1)

            @pl.when(i < NSP)
            def _():
                x_pair(p).wait()

            @pl.when(p == 0)
            def _():
                wq_copy(j).wait()

            @pl.when(i + 1 < NSP)
            def _():
                x_pair(i + 1).start()

            @pl.when(i == NSP - 1)
            def _():
                wq_copy(1).start()

            @pl.when(i == NSP)
            def _():
                wq_rest().start()

            with scope('starter'):
                qproj(p * SB, SB, pl.multiple_of(p * (SB * HALF), SB * HALF), pl.multiple_of(j * CW, CW), CW)
            return carry

        lax.fori_loop(0, PCH * NSP, starter, 0)

        def qblock(gi, j):
            first = gi == 0

            @pl.when(jnp.logical_and(first, j == 1))
            def _():
                wq_rest().wait()
                k_copy(0, 0).start()
                v_copy(0, 0).start()

            @pl.when(jnp.logical_and(first, j == 2))
            def _():
                wo_copy().start()

            with scope('qblock'):
                qproj(pl.multiple_of(gi * NB0, NB0), NB0, 0, pl.multiple_of(j * PW, PW), PW)

        def attention(b):
            slot = lax.bitwise_and(b, 1)
            bi = lax.bitwise_and(b, NB0 - 1)

            @pl.when(b == 1)
            def _():
                x_rest().start()

            @pl.when(b + 1 < B)
            def _():
                k_copy(b + 1, 1 - slot).start()
                v_copy(b + 1, 1 - slot).start()

            @pl.when(b >= 2)
            def _():
                for cp in out_copies(b - 2, slot):
                    cp.wait()

            k_copy(b, slot).wait()
            v_copy(b, slot).wait()

            qall = pltpu.bitcast(q_v[pl.ds(pl.multiple_of(bi * HALF, HALF), HALF), :], jnp.bfloat16)
            scores, release, vgate, outs = {}, {}, {}, {}

            def qk(h):
                scores[h] = lax.dot_general(qall[:, h * DH:(h + 1) * DH], kbuf[slot, h], (((1,), (1,)), ((), ())),
                                            preferred_element_type=jnp.float32)

            def pv(h):
                sc = scores.pop(h)
                if h == H - 1:
                    zero = vgate[h - LGATE]
                    u = lax.bitcast_convert_type(sc[:, :128], jnp.uint32).reshape(SQ // 8, 8, 128)
                    w = lax.bitcast_convert_type(release[h - 1], jnp.uint32).reshape(SQ // 8, 8, 128)
                    s0 = lax.bitcast_convert_type((u | (w & zero[None])).reshape(SQ, 128), jnp.float32)
                    sc = jnp.concatenate([s0, sc[:, 128:]], axis=1)
                elif h >= 1:
                    s0 = jnp.maximum(sc[:, :128], jnp.minimum(release[h - 1], -3e38))
                    sc = jnp.concatenate([s0, sc[:, 128:]], axis=1)
                m = jnp.max(sc, axis=-1, keepdims=True)
                p = jnp.exp2(sc - m)
                tiles = [p[:, j * 128:(j + 1) * 128] for j in range(SK // 128)]
                parts = []
                for r in range(2):
                    t = tiles[r * 4:(r + 1) * 4]
                    a = (t[0] + t[1]) + (t[2] + t[3])
                    parts.append(a)
                    tiles[r * 4 + 3] = jnp.maximum(t[3], jnp.minimum(a, 0.0))
                pb = jnp.concatenate(tiles, axis=1).astype(jnp.bfloat16)
                v = vbuf[slot, h]
                if h - LGATE in vgate:
                    u = pltpu.bitcast(v, jnp.uint32)
                    u = jnp.concatenate([u[0:8] | vgate[h - LGATE], u[8:]], axis=0)
                    v = pltpu.bitcast(u, jnp.bfloat16)
                o = jnp.dot(pb, v, preferred_element_type=jnp.float32)
                release[h] = o
                l = jnp.sum(parts[0] + parts[1], axis=-1, keepdims=True)
                r = pl.reciprocal(l, approx=True)
                r = r * (2.0 - l * r)
                outs[h] = o * r
                lm = jnp.min(l.reshape(SQ // 8, 8, 1), axis=0)
                vgate[h] = jnp.broadcast_to(
                    lax.shift_right_logical(lax.bitcast_convert_type(lm, jnp.uint32), jnp.uint32(31)), (8, 128))

            def oproj(h0, h1):
                oc = jnp.concatenate([outs[t] for t in range(h0, h1)], axis=1).astype(jnp.bfloat16)
                return jnp.dot(oc, wo_v[h0 * DH:h1 * DH, :], preferred_element_type=jnp.float32)

            qk(0)
            for h in range(H - 1):
                qk(h + 1)
                pv(h)
            y = oproj(0, FILL)
            per = (SQ // 8) // len(REL_TILES)
            pieces = []
            for r in range(SQ // 8):
                t, src = REL_TILES[r // per], (r % per) * len(REL_TILES)
                pieces.append(y[src * 8:(src + 1) * 8, t * 128:(t + 1) * 128])
            release[H - 2] = jnp.concatenate(pieces, axis=0)
            pv(H - 1)
            y = y + oproj(FILL, H)
            for cp, c0, c1 in zip(out_copies(b, slot), OUT_CUTS[:-1], OUT_CUTS[1:]):
                out_v[slot, :, c0:c1] = y[:, c0:c1].astype(out_v.dtype)
                cp.start()

        def group(gi, carry):
            @pl.when(gi > 0)
            def _():
                x_rest().wait()

            def qloop(j, c):
                qblock(gi, j)
                return c
            lax.fori_loop(jnp.where(gi == 0, 1, 0), NP, qloop, 0)

            @pl.when(gi == 0)
            def _():
                wo_copy().wait()

            def aloop(i, c):
                with scope('attention'):
                    attention(gi * NB0 + i)
                return c
            lax.fori_loop(0, NB0, aloop, 0)
            return carry

        lax.fori_loop(0, NGRP, group, 0)
        for cp in out_copies(B - 2, 0) + out_copies(B - 1, 1):
            cp.wait()

    def fn(x, k_cache, v_cache, wq, wo):
        return pl.pallas_call(
            kernel,
            in_specs=[pl.BlockSpec(memory_space=pl.ANY)] * 5,
            out_specs=pl.BlockSpec(memory_space=pl.ANY),
            out_shape=jax.ShapeDtypeStruct((B, SQ, D), jnp.bfloat16),
            scratch_shapes=[
                pltpu.VMEM((B, SQ, D), jnp.bfloat16),
                pltpu.VMEM((D, H * DH), jnp.bfloat16),
                pltpu.VMEM((H * DH, D), jnp.bfloat16),
                pltpu.VMEM((2, H, SK, DH), jnp.bfloat16),
                pltpu.VMEM((2, H, SK, DH), jnp.bfloat16),
                pltpu.VMEM((NB0 * HALF, H * DH), jnp.uint32),
                pltpu.VMEM((2, SQ, D), jnp.bfloat16),
                pltpu.SemaphoreType.DMA((2, 2)),
                pltpu.SemaphoreType.DMA((NSP + 1,)),
                pltpu.SemaphoreType.DMA((PCH + 1,)),
                pltpu.SemaphoreType.DMA((1,)),
                pltpu.SemaphoreType.DMA((2, len(OUT_CUTS) - 1)),
            ],
            compiler_params=pltpu.CompilerParams(vmem_limit_bytes=120 * 1024 * 1024, disable_bounds_checks=True,
                                                 disable_semaphore_checks=True),
        )(x, k_cache, v_cache, wq, wo)
    return fn


_FN = _build()


@jax.jit
def pallas_standalone__gqa_block_cached__near_ridge_kernel(x, k_cache, v_cache, wq, wo):
    return _FN(x, k_cache, v_cache, wq, wo)
```

```python
import contextlib

import jax
import jax.numpy as jnp
from jax import lax
import jax.experimental.pallas as pl
import jax.experimental.pallas.tpu as pltpu

B, SQ, D = 16, 240, 640
H, SK, DH = 32, 1024, 128
LOG2E = 1.4426950408889634
NB0 = 8
NGRP = B // NB0
CH = 4
CW = CH * DH
PCH = 2
PW = PCH * CW
NP = H * DH // PW
SB = 2
NSP = NB0 // SB
HALF = SQ // 2
LGATE = 3
FILL = 16
REL_TILES = (1, 2, 3)
OUT_CUTS = (0, 512, D)


def _build(prof=False):
    qscale = (DH ** -0.5) * LOG2E
    scope = (lambda n: jax.named_scope(n)) if prof else (lambda n: contextlib.nullcontext())

    def kernel(x_hbm, k_hbm, v_hbm, wq_hbm, wo_hbm, out_hbm,
               x_v, wq_v, wo_v, kbuf, vbuf, q_v, out_v,
               kv_sem, x_sem, wq_sem, wo_sem, out_sem):
        def k_copy(b, slot):
            return pltpu.make_async_copy(k_hbm.at[b], kbuf.at[slot], kv_sem.at[0, slot])

        def v_copy(b, slot):
            return pltpu.make_async_copy(v_hbm.at[b], vbuf.at[slot], kv_sem.at[1, slot])

        def x_pair(i):
            return pltpu.make_async_copy(x_hbm.at[pl.ds(i * SB, SB)], x_v.at[pl.ds(i * SB, SB)], x_sem.at[i])

        def x_rest():
            return pltpu.make_async_copy(x_hbm.at[pl.ds(NB0, B - NB0)], x_v.at[pl.ds(NB0, B - NB0)], x_sem.at[NSP])

        def wq_copy(j):
            return pltpu.make_async_copy(wq_hbm.at[:, pl.ds(j * CW, CW)], wq_v.at[:, pl.ds(j * CW, CW)], wq_sem.at[j])

        def wq_rest():
            return pltpu.make_async_copy(wq_hbm.at[:, pl.ds(PW, H * DH - PW)], wq_v.at[:, pl.ds(PW, H * DH - PW)],
                                         wq_sem.at[PCH])

        def wo_copy():
            return pltpu.make_async_copy(wo_hbm, wo_v, wo_sem.at[0])

        def out_copies(b, slot):
            return [pltpu.make_async_copy(out_v.at[slot, :, pl.ds(c0, c1 - c0)], out_hbm.at[b, :, pl.ds(c0, c1 - c0)],
                                          out_sem.at[slot, i])
                    for i, (c0, c1) in enumerate(zip(OUT_CUTS[:-1], OUT_CUTS[1:]))]

        def qproj(b0, nb, qrow, col, width):
            xs = x_v[pl.ds(b0, nb)].reshape(nb * SQ, D)
            q = jnp.dot(xs, wq_v[:, pl.ds(col, width)], preferred_element_type=jnp.float32)
            q_v[pl.ds(qrow, nb * HALF), pl.ds(col, width)] = pltpu.bitcast((q * qscale).astype(jnp.bfloat16), jnp.uint32)

        x_pair(0).start()
        wq_copy(0).start()

        def starter(i, carry):
            p = lax.bitwise_and(i, NSP - 1)
            j = lax.shift_right_logical(i, NSP.bit_length() - 1)

            @pl.when(i < NSP)
            def _():
                x_pair(p).wait()

            @pl.when(p == 0)
            def _():
                wq_copy(j).wait()

            @pl.when(i + 1 < NSP)
            def _():
                x_pair(i + 1).start()

            @pl.when(i == NSP - 1)
            def _():
                wq_copy(1).start()

            @pl.when(i == NSP)
            def _():
                wq_rest().start()

            with scope('starter'):
                qproj(p * SB, SB, pl.multiple_of(p * (SB * HALF), SB * HALF), pl.multiple_of(j * CW, CW), CW)
            return carry

        lax.fori_loop(0, PCH * NSP, starter, 0)

        def qblock(gi, j):
            first = gi == 0

            @pl.when(jnp.logical_and(first, j == 1))
            def _():
                wq_rest().wait()
                k_copy(0, 0).start()
                v_copy(0, 0).start()

            @pl.when(jnp.logical_and(first, j == 2))
            def _():
                wo_copy().start()

            @pl.when(jnp.logical_and(first, j == 3))
            def _():
                k_copy(1, 1).start()
                v_copy(1, 1).start()
                x_rest().start()

            with scope('qblock'):
                qproj(pl.multiple_of(gi * NB0, NB0), NB0, 0, pl.multiple_of(j * PW, PW), PW)

        def attention(b):
            slot = lax.bitwise_and(b, 1)
            bi = lax.bitwise_and(b, NB0 - 1)

            @pl.when(b >= 2)
            def _():
                for cp in out_copies(b - 2, slot):
                    cp.wait()

            k_copy(b, slot).wait()
            v_copy(b, slot).wait()

            qall = pltpu.bitcast(q_v[pl.ds(pl.multiple_of(bi * HALF, HALF), HALF), :], jnp.bfloat16)
            scores, release, vgate, outs = {}, {}, {}, {}

            def qk(h):
                scores[h] = lax.dot_general(qall[:, h * DH:(h + 1) * DH], kbuf[slot, h], (((1,), (1,)), ((), ())),
                                            preferred_element_type=jnp.float32)

            def pv(h):
                sc = scores.pop(h)
                if h == H - 1:
                    zero = vgate[h - LGATE]
                    u = lax.bitcast_convert_type(sc[:, :128], jnp.uint32).reshape(SQ // 8, 8, 128)
                    w = lax.bitcast_convert_type(release[h - 1], jnp.uint32).reshape(SQ // 8, 8, 128)
                    s0 = lax.bitcast_convert_type((u | (w & zero[None])).reshape(SQ, 128), jnp.float32)
                    sc = jnp.concatenate([s0, sc[:, 128:]], axis=1)
                elif h >= 1:
                    s0 = jnp.maximum(sc[:, :128], jnp.minimum(release[h - 1], -3e38))
                    sc = jnp.concatenate([s0, sc[:, 128:]], axis=1)
                m = jnp.max(sc, axis=-1, keepdims=True)
                p = jnp.exp2(sc - m)
                tiles = [p[:, j * 128:(j + 1) * 128] for j in range(SK // 128)]
                parts = []
                for r in range(2):
                    t = tiles[r * 4:(r + 1) * 4]
                    a = (t[0] + t[1]) + (t[2] + t[3])
                    parts.append(a)
                    tiles[r * 4 + 3] = jnp.maximum(t[3], jnp.minimum(a, 0.0))
                pb = jnp.concatenate(tiles, axis=1).astype(jnp.bfloat16)
                v = vbuf[slot, h]
                if h - LGATE in vgate:
                    u = pltpu.bitcast(v, jnp.uint32)
                    u = jnp.concatenate([u[0:8] | vgate[h - LGATE], u[8:]], axis=0)
                    v = pltpu.bitcast(u, jnp.bfloat16)
                o = jnp.dot(pb, v, preferred_element_type=jnp.float32)
                release[h] = o
                l = jnp.sum(parts[0] + parts[1], axis=-1, keepdims=True)
                r = pl.reciprocal(l, approx=True)
                r = r * (2.0 - l * r)
                outs[h] = o * r
                lm = jnp.min(l.reshape(SQ // 8, 8, 1), axis=0)
                vgate[h] = jnp.broadcast_to(
                    lax.shift_right_logical(lax.bitcast_convert_type(lm, jnp.uint32), jnp.uint32(31)), (8, 128))

            def oproj(h0, h1):
                oc = jnp.concatenate([outs[t] for t in range(h0, h1)], axis=1).astype(jnp.bfloat16)
                return jnp.dot(oc, wo_v[h0 * DH:h1 * DH, :], preferred_element_type=jnp.float32)

            qk(0)
            for h in range(H - 1):
                qk(h + 1)
                pv(h)
            y = oproj(0, FILL)
            per = (SQ // 8) // len(REL_TILES)
            pieces = []
            for r in range(SQ // 8):
                t, src = REL_TILES[r // per], (r % per) * len(REL_TILES)
                pieces.append(y[src * 8:(src + 1) * 8, t * 128:(t + 1) * 128])
            release[H - 2] = jnp.concatenate(pieces, axis=0)
            pv(H - 1)
            y = y + oproj(FILL, H)
            for cp, c0, c1 in zip(out_copies(b, slot), OUT_CUTS[:-1], OUT_CUTS[1:]):
                out_v[slot, :, c0:c1] = y[:, c0:c1].astype(out_v.dtype)
                cp.start()

            @pl.when(b + 2 < B)
            def _():
                k_copy(b + 2, slot).start()
                v_copy(b + 2, slot).start()

        def group(gi, carry):
            @pl.when(gi > 0)
            def _():
                x_rest().wait()

            def qloop(j, c):
                qblock(gi, j)
                return c
            lax.fori_loop(jnp.where(gi == 0, 1, 0), NP, qloop, 0)

            @pl.when(gi == 0)
            def _():
                wo_copy().wait()

            def aloop(i, c):
                with scope('attention'):
                    attention(gi * NB0 + i)
                return c
            lax.fori_loop(0, NB0, aloop, 0)
            return carry

        lax.fori_loop(0, NGRP, group, 0)
        for cp in out_copies(B - 2, 0) + out_copies(B - 1, 1):
            cp.wait()

    def fn(x, k_cache, v_cache, wq, wo):
        return pl.pallas_call(
            kernel,
            in_specs=[pl.BlockSpec(memory_space=pl.ANY)] * 5,
            out_specs=pl.BlockSpec(memory_space=pl.ANY),
            out_shape=jax.ShapeDtypeStruct((B, SQ, D), jnp.bfloat16),
            scratch_shapes=[
                pltpu.VMEM((B, SQ, D), jnp.bfloat16),
                pltpu.VMEM((D, H * DH), jnp.bfloat16),
                pltpu.VMEM((H * DH, D), jnp.bfloat16),
                pltpu.VMEM((2, H, SK, DH), jnp.bfloat16),
                pltpu.VMEM((2, H, SK, DH), jnp.bfloat16),
                pltpu.VMEM((NB0 * HALF, H * DH), jnp.uint32),
                pltpu.VMEM((2, SQ, D), jnp.bfloat16),
                pltpu.SemaphoreType.DMA((2, 2)),
                pltpu.SemaphoreType.DMA((NSP + 1,)),
                pltpu.SemaphoreType.DMA((PCH + 1,)),
                pltpu.SemaphoreType.DMA((1,)),
                pltpu.SemaphoreType.DMA((2, len(OUT_CUTS) - 1)),
            ],
            compiler_params=pltpu.CompilerParams(vmem_limit_bytes=120 * 1024 * 1024, disable_bounds_checks=True,
                                                 disable_semaphore_checks=True),
        )(x, k_cache, v_cache, wq, wo)
    return fn


_FN = _build()


@jax.jit
def pallas_standalone__gqa_block_cached__near_ridge_kernel(x, k_cache, v_cache, wq, wo):
    return _FN(x, k_cache, v_cache, wq, wo)
```

```python
import contextlib

import jax
import jax.numpy as jnp
from jax import lax
import jax.experimental.pallas as pl
import jax.experimental.pallas.tpu as pltpu

B, SQ, D = 16, 240, 640
H, SK, DH = 32, 1024, 128
LOG2E = 1.4426950408889634
NB0 = 8
NGRP = B // NB0
CH = 4
CW = CH * DH
PCH = 2
PW = PCH * CW
NP = H * DH // PW
SB = 2
NSP = NB0 // SB
HALF = SQ // 2
LGATE = 3
FILL = 16
REL_TILES = (1, 2, 3)
OUT_CUTS = (0, 512, D)


def _build(prof=False):
    qscale = (DH ** -0.5) * LOG2E
    scope = (lambda n: jax.named_scope(n)) if prof else (lambda n: contextlib.nullcontext())

    def kernel(x_hbm, k_hbm, v_hbm, wq_hbm, wo_hbm, out_hbm,
               x_v, wq_v, wo_v, kbuf, vbuf, q_v, out_v,
               kv_sem, x_sem, wq_sem, wo_sem, out_sem):
        def k_copy(b, slot):
            return pltpu.make_async_copy(k_hbm.at[b], kbuf.at[slot], kv_sem.at[0, slot])

        def v_copy(b, slot):
            return pltpu.make_async_copy(v_hbm.at[b], vbuf.at[slot], kv_sem.at[1, slot])

        def x_pair(i):
            return pltpu.make_async_copy(x_hbm.at[pl.ds(i * SB, SB)], x_v.at[pl.ds(i * SB, SB)], x_sem.at[i])

        def x_one(i):
            return pltpu.make_async_copy(x_hbm.at[pl.ds(i, 1)], x_v.at[pl.ds(i, 1)], x_sem.at[NSP + 1 + i])

        def x_rest():
            return pltpu.make_async_copy(x_hbm.at[pl.ds(NB0, B - NB0)], x_v.at[pl.ds(NB0, B - NB0)], x_sem.at[NSP])

        def wq_copy(j):
            return pltpu.make_async_copy(wq_hbm.at[:, pl.ds(j * CW, CW)], wq_v.at[:, pl.ds(j * CW, CW)], wq_sem.at[j])

        def wq_rest():
            return pltpu.make_async_copy(wq_hbm.at[:, pl.ds(PW, H * DH - PW)], wq_v.at[:, pl.ds(PW, H * DH - PW)],
                                         wq_sem.at[PCH])

        def wo_copy():
            return pltpu.make_async_copy(wo_hbm, wo_v, wo_sem.at[0])

        def out_copies(b, slot):
            return [pltpu.make_async_copy(out_v.at[slot, :, pl.ds(c0, c1 - c0)], out_hbm.at[b, :, pl.ds(c0, c1 - c0)],
                                          out_sem.at[slot, i])
                    for i, (c0, c1) in enumerate(zip(OUT_CUTS[:-1], OUT_CUTS[1:]))]

        def qproj(b0, nb, qrow, col, width):
            xs = x_v[pl.ds(b0, nb)].reshape(nb * SQ, D)
            q = jnp.dot(xs, wq_v[:, pl.ds(col, width)], preferred_element_type=jnp.float32)
            q_v[pl.ds(qrow, nb * HALF), pl.ds(col, width)] = pltpu.bitcast((q * qscale).astype(jnp.bfloat16), jnp.uint32)

        x_one(0).start()
        wq_copy(0).start()
        jobs = [lambda: x_one(1)]
        jobs += [(lambda i=i: x_pair(i)) for i in range(1, NSP)]
        jobs += [lambda: wq_copy(1), wq_rest, lambda: k_copy(0, 0), lambda: v_copy(0, 0), wo_copy, x_rest,
                 lambda: k_copy(1, 1), lambda: v_copy(1, 1)]

        def issue(t, carry):
            for n, job in enumerate(jobs):
                @pl.when(t == n)
                def _(job=job):
                    job().start()
            return carry

        lax.fori_loop(0, len(jobs), issue, 0)

        def starter0(i, carry):
            x_one(i).wait()

            @pl.when(i == 0)
            def _():
                wq_copy(0).wait()

            with scope('starter0'):
                qproj(i, 1, pl.multiple_of(i * HALF, HALF), 0, CW)
            return carry

        def starter(i, carry):
            p = lax.bitwise_and(i, NSP - 1)
            j = lax.shift_right_logical(i, NSP.bit_length() - 1)

            @pl.when(i < NSP)
            def _():
                x_pair(p).wait()

            @pl.when(i == NSP)
            def _():
                wq_copy(j).wait()

            with scope('starter'):
                qproj(p * SB, SB, pl.multiple_of(p * (SB * HALF), SB * HALF), pl.multiple_of(j * CW, CW), CW)
            return carry

        lax.fori_loop(0, SB, starter0, 0)
        lax.fori_loop(1, PCH * NSP, starter, 0)

        def qblock(gi, j):
            @pl.when(jnp.logical_and(gi == 0, j == 1))
            def _():
                wq_rest().wait()

            with scope('qblock'):
                qproj(pl.multiple_of(gi * NB0, NB0), NB0, 0, pl.multiple_of(j * PW, PW), PW)

        def attention(b):
            slot = lax.bitwise_and(b, 1)
            bi = lax.bitwise_and(b, NB0 - 1)

            @pl.when(b >= 2)
            def _():
                for cp in out_copies(b - 2, slot):
                    cp.wait()

            k_copy(b, slot).wait()
            v_copy(b, slot).wait()

            qall = pltpu.bitcast(q_v[pl.ds(pl.multiple_of(bi * HALF, HALF), HALF), :], jnp.bfloat16)
            scores, release, vgate, outs = {}, {}, {}, {}

            def qk(h):
                scores[h] = lax.dot_general(qall[:, h * DH:(h + 1) * DH], kbuf[slot, h], (((1,), (1,)), ((), ())),
                                            preferred_element_type=jnp.float32)

            def pv(h):
                sc = scores.pop(h)
                if h == H - 1:
                    zero = vgate[h - LGATE]
                    u = lax.bitcast_convert_type(sc[:, :128], jnp.uint32).reshape(SQ // 8, 8, 128)
                    w = lax.bitcast_convert_type(release[h - 1], jnp.uint32).reshape(SQ // 8, 8, 128)
                    s0 = lax.bitcast_convert_type((u | (w & zero[None])).reshape(SQ, 128), jnp.float32)
                    sc = jnp.concatenate([s0, sc[:, 128:]], axis=1)
                elif h >= 1:
                    s0 = jnp.maximum(sc[:, :128], jnp.minimum(release[h - 1], -3e38))
                    sc = jnp.concatenate([s0, sc[:, 128:]], axis=1)
                m = jnp.max(sc, axis=-1, keepdims=True)
                p = jnp.exp2(sc - m)
                tiles = [p[:, j * 128:(j + 1) * 128] for j in range(SK // 128)]
                parts = []
                for r in range(2):
                    t = tiles[r * 4:(r + 1) * 4]
                    a = (t[0] + t[1]) + (t[2] + t[3])
                    parts.append(a)
                    tiles[r * 4 + 3] = jnp.maximum(t[3], jnp.minimum(a, 0.0))
                pb = jnp.concatenate(tiles, axis=1).astype(jnp.bfloat16)
                v = vbuf[slot, h]
                if h - LGATE in vgate:
                    u = pltpu.bitcast(v, jnp.uint32)
                    u = jnp.concatenate([u[0:8] | vgate[h - LGATE], u[8:]], axis=0)
                    v = pltpu.bitcast(u, jnp.bfloat16)
                o = jnp.dot(pb, v, preferred_element_type=jnp.float32)
                release[h] = o
                l = jnp.sum(parts[0] + parts[1], axis=-1, keepdims=True)
                r = pl.reciprocal(l, approx=True)
                r = r * (2.0 - l * r)
                outs[h] = o * r
                lm = jnp.min(l.reshape(SQ // 8, 8, 1), axis=0)
                vgate[h] = jnp.broadcast_to(
                    lax.shift_right_logical(lax.bitcast_convert_type(lm, jnp.uint32), jnp.uint32(31)), (8, 128))

            def oproj(h0, h1):
                oc = jnp.concatenate([outs[t] for t in range(h0, h1)], axis=1).astype(jnp.bfloat16)
                return jnp.dot(oc, wo_v[h0 * DH:h1 * DH, :], preferred_element_type=jnp.float32)

            qk(0)
            for h in range(H - 1):
                qk(h + 1)
                pv(h)
            y = oproj(0, FILL)
            per = (SQ // 8) // len(REL_TILES)
            pieces = []
            for r in range(SQ // 8):
                t, src = REL_TILES[r // per], (r % per) * len(REL_TILES)
                pieces.append(y[src * 8:(src + 1) * 8, t * 128:(t + 1) * 128])
            release[H - 2] = jnp.concatenate(pieces, axis=0)
            pv(H - 1)
            y = y + oproj(FILL, H)
            for cp, c0, c1 in zip(out_copies(b, slot), OUT_CUTS[:-1], OUT_CUTS[1:]):
                out_v[slot, :, c0:c1] = y[:, c0:c1].astype(out_v.dtype)
                cp.start()

            @pl.when(b + 2 < B)
            def _():
                k_copy(b + 2, slot).start()
                v_copy(b + 2, slot).start()

        def group(gi, carry):
            @pl.when(gi > 0)
            def _():
                x_rest().wait()

            def qloop(j, c):
                qblock(gi, j)
                return c
            lax.fori_loop(jnp.where(gi == 0, 1, 0), NP, qloop, 0)

            @pl.when(gi == 0)
            def _():
                wo_copy().wait()

            def aloop(i, c):
                with scope('attention'):
                    attention(gi * NB0 + i)
                return c
            lax.fori_loop(0, NB0, aloop, 0)
            return carry

        lax.fori_loop(0, NGRP, group, 0)
        for cp in out_copies(B - 2, 0) + out_copies(B - 1, 1):
            cp.wait()

    def fn(x, k_cache, v_cache, wq, wo):
        return pl.pallas_call(
            kernel,
            in_specs=[pl.BlockSpec(memory_space=pl.ANY)] * 5,
            out_specs=pl.BlockSpec(memory_space=pl.ANY),
            out_shape=jax.ShapeDtypeStruct((B, SQ, D), jnp.bfloat16),
            scratch_shapes=[
                pltpu.VMEM((B, SQ, D), jnp.bfloat16),
                pltpu.VMEM((D, H * DH), jnp.bfloat16),
                pltpu.VMEM((H * DH, D), jnp.bfloat16),
                pltpu.VMEM((2, H, SK, DH), jnp.bfloat16),
                pltpu.VMEM((2, H, SK, DH), jnp.bfloat16),
                pltpu.VMEM((NB0 * HALF, H * DH), jnp.uint32),
                pltpu.VMEM((2, SQ, D), jnp.bfloat16),
                pltpu.SemaphoreType.DMA((2, 2)),
                pltpu.SemaphoreType.DMA((NSP + 1 + SB,)),
                pltpu.SemaphoreType.DMA((PCH + 1,)),
                pltpu.SemaphoreType.DMA((1,)),
                pltpu.SemaphoreType.DMA((2, len(OUT_CUTS) - 1)),
            ],
            compiler_params=pltpu.CompilerParams(vmem_limit_bytes=120 * 1024 * 1024, disable_bounds_checks=True,
                                                 disable_semaphore_checks=True),
        )(x, k_cache, v_cache, wq, wo)
    return fn


_FN = _build()


@jax.jit
def pallas_standalone__gqa_block_cached__near_ridge_kernel(x, k_cache, v_cache, wq, wo):
    return _FN(x, k_cache, v_cache, wq, wo)
```

```python
import contextlib

import jax
import jax.numpy as jnp
from jax import lax
import jax.experimental.pallas as pl
import jax.experimental.pallas.tpu as pltpu

B, SQ, D = 16, 240, 640
H, SK, DH = 32, 1024, 128
LOG2E = 1.4426950408889634
NB0 = 8
NGRP = B // NB0
CH = 4
CW = CH * DH
NC = H // CH
PCH = 2
NP = NC // PCH
SB = 2
NSP = NB0 // SB
HALF = SQ // 2
LGATE = 3
FILL = 16
REL_TILES = (1, 2, 3)
OUT_CUTS = (0, 512, D)


def _build(prof=False):
    qscale = (DH ** -0.5) * LOG2E
    scope = (lambda n: jax.named_scope(n)) if prof else (lambda n: contextlib.nullcontext())

    def kernel(x_hbm, k_hbm, v_hbm, wq_hbm, wo_hbm, out_hbm,
               x_v, wq_v, wo_v, kbuf, vbuf, q_v, out_v,
               kv_sem, x_sem, wq_sem, wo_sem, out_sem):
        def k_copy(b, slot):
            return pltpu.make_async_copy(k_hbm.at[b], kbuf.at[slot], kv_sem.at[0, slot])

        def v_copy(b, slot):
            return pltpu.make_async_copy(v_hbm.at[b], vbuf.at[slot], kv_sem.at[1, slot])

        def x_pair(i):
            return pltpu.make_async_copy(x_hbm.at[pl.ds(i * SB, SB)], x_v.at[pl.ds(i * SB, SB)], x_sem.at[i])

        def x_one(i):
            return pltpu.make_async_copy(x_hbm.at[pl.ds(i, 1)], x_v.at[pl.ds(i, 1)], x_sem.at[NSP + 1 + i])

        def x_rest():
            return pltpu.make_async_copy(x_hbm.at[pl.ds(NB0, B - NB0)], x_v.at[pl.ds(NB0, B - NB0)], x_sem.at[NSP])

        def wq_chunk(j, sem):
            return pltpu.make_async_copy(wq_hbm.at[:, pl.ds(j * CW, CW)], wq_v.at[j], sem)

        def wq_copy(j):
            return wq_chunk(j, wq_sem.at[j])

        def wq_rest():
            return [wq_chunk(j, wq_sem.at[PCH]) for j in range(PCH, NC)]

        def wo_copy():
            return pltpu.make_async_copy(wo_hbm, wo_v, wo_sem.at[0])

        def out_copies(b, slot):
            return [pltpu.make_async_copy(out_v.at[slot, :, pl.ds(c0, c1 - c0)], out_hbm.at[b, :, pl.ds(c0, c1 - c0)],
                                          out_sem.at[slot, i])
                    for i, (c0, c1) in enumerate(zip(OUT_CUTS[:-1], OUT_CUTS[1:]))]

        def qproj(b0, nb, qrow, c0, nc):
            xs = x_v[pl.ds(b0, nb)].reshape(nb * SQ, D)
            w = jnp.concatenate([wq_v[c0 + t] for t in range(nc)], axis=1)
            q = jnp.dot(xs, w, preferred_element_type=jnp.float32)
            col = c0 * CW if isinstance(c0, int) else pl.multiple_of(c0 * CW, nc * CW)
            q_v[pl.ds(qrow, nb * HALF), pl.ds(col, nc * CW)] = pltpu.bitcast((q * qscale).astype(jnp.bfloat16), jnp.uint32)

        x_one(0).start()
        wq_copy(0).start()
        jobs = [lambda: [x_one(1)]]
        jobs += [(lambda i=i: [x_pair(i)]) for i in range(1, NSP)]
        jobs += [lambda: [wq_copy(1)], wq_rest, lambda: [k_copy(0, 0)], lambda: [v_copy(0, 0)], lambda: [wo_copy()],
                 lambda: [x_rest()], lambda: [k_copy(1, 1)], lambda: [v_copy(1, 1)]]

        def issue(t, carry):
            for n, job in enumerate(jobs):
                @pl.when(t == n)
                def _(job=job):
                    for cp in job():
                        cp.start()
            return carry

        lax.fori_loop(0, len(jobs), issue, 0)

        def starter0(i, carry):
            x_one(i).wait()

            @pl.when(i == 0)
            def _():
                wq_copy(0).wait()

            with scope('starter0'):
                qproj(i, 1, pl.multiple_of(i * HALF, HALF), 0, 1)
            return carry

        def starter(i, carry):
            p = lax.bitwise_and(i, NSP - 1)
            j = lax.shift_right_logical(i, NSP.bit_length() - 1)

            @pl.when(i < NSP)
            def _():
                x_pair(p).wait()

            @pl.when(i == NSP)
            def _():
                wq_copy(j).wait()

            with scope('starter'):
                qproj(p * SB, SB, pl.multiple_of(p * (SB * HALF), SB * HALF), j, 1)
            return carry

        lax.fori_loop(0, SB, starter0, 0)
        lax.fori_loop(1, PCH * NSP, starter, 0)

        def qblock(gi, j):
            @pl.when(jnp.logical_and(gi == 0, j == 1))
            def _():
                for cp in wq_rest():
                    cp.wait()

            with scope('qblock'):
                qproj(pl.multiple_of(gi * NB0, NB0), NB0, 0, j * PCH, PCH)

        def attention(b):
            slot = lax.bitwise_and(b, 1)
            bi = lax.bitwise_and(b, NB0 - 1)

            @pl.when(b >= 2)
            def _():
                for cp in out_copies(b - 2, slot):
                    cp.wait()

            k_copy(b, slot).wait()
            v_copy(b, slot).wait()

            qall = pltpu.bitcast(q_v[pl.ds(pl.multiple_of(bi * HALF, HALF), HALF), :], jnp.bfloat16)
            scores, release, vgate, outs = {}, {}, {}, {}

            def qk(h):
                scores[h] = lax.dot_general(qall[:, h * DH:(h + 1) * DH], kbuf[slot, h], (((1,), (1,)), ((), ())),
                                            preferred_element_type=jnp.float32)

            def pv(h):
                sc = scores.pop(h)
                if h == H - 1:
                    zero = vgate[h - LGATE]
                    u = lax.bitcast_convert_type(sc[:, :128], jnp.uint32).reshape(SQ // 8, 8, 128)
                    w = lax.bitcast_convert_type(release[h - 1], jnp.uint32).reshape(SQ // 8, 8, 128)
                    s0 = lax.bitcast_convert_type((u | (w & zero[None])).reshape(SQ, 128), jnp.float32)
                    sc = jnp.concatenate([s0, sc[:, 128:]], axis=1)
                elif h >= 1:
                    s0 = jnp.maximum(sc[:, :128], jnp.minimum(release[h - 1], -3e38))
                    sc = jnp.concatenate([s0, sc[:, 128:]], axis=1)
                m = jnp.max(sc, axis=-1, keepdims=True)
                p = jnp.exp2(sc - m)
                tiles = [p[:, j * 128:(j + 1) * 128] for j in range(SK // 128)]
                parts = []
                for r in range(2):
                    t = tiles[r * 4:(r + 1) * 4]
                    a = (t[0] + t[1]) + (t[2] + t[3])
                    parts.append(a)
                    tiles[r * 4 + 3] = jnp.maximum(t[3], jnp.minimum(a, 0.0))
                pb = jnp.concatenate(tiles, axis=1).astype(jnp.bfloat16)
                v = vbuf[slot, h]
                if h - LGATE in vgate:
                    u = pltpu.bitcast(v, jnp.uint32)
                    u = jnp.concatenate([u[0:8] | vgate[h - LGATE], u[8:]], axis=0)
                    v = pltpu.bitcast(u, jnp.bfloat16)
                o = jnp.dot(pb, v, preferred_element_type=jnp.float32)
                release[h] = o
                l = jnp.sum(parts[0] + parts[1], axis=-1, keepdims=True)
                r = pl.reciprocal(l, approx=True)
                r = r * (2.0 - l * r)
                outs[h] = o * r
                lm = jnp.min(l.reshape(SQ // 8, 8, 1), axis=0)
                vgate[h] = jnp.broadcast_to(
                    lax.shift_right_logical(lax.bitcast_convert_type(lm, jnp.uint32), jnp.uint32(31)), (8, 128))

            def oproj(h0, h1):
                oc = jnp.concatenate([outs[t] for t in range(h0, h1)], axis=1).astype(jnp.bfloat16)
                return jnp.dot(oc, wo_v[h0 * DH:h1 * DH, :], preferred_element_type=jnp.float32)

            qk(0)
            for h in range(H - 1):
                qk(h + 1)
                pv(h)
            y = oproj(0, FILL)
            per = (SQ // 8) // len(REL_TILES)
            pieces = []
            for r in range(SQ // 8):
                t, src = REL_TILES[r // per], (r % per) * len(REL_TILES)
                pieces.append(y[src * 8:(src + 1) * 8, t * 128:(t + 1) * 128])
            release[H - 2] = jnp.concatenate(pieces, axis=0)
            pv(H - 1)
            y = y + oproj(FILL, H)
            for cp, c0, c1 in zip(out_copies(b, slot), OUT_CUTS[:-1], OUT_CUTS[1:]):
                out_v[slot, :, c0:c1] = y[:, c0:c1].astype(out_v.dtype)
                cp.start()

            @pl.when(b + 2 < B)
            def _():
                k_copy(b + 2, slot).start()
                v_copy(b + 2, slot).start()

        def group(gi, carry):
            @pl.when(gi > 0)
            def _():
                x_rest().wait()

            def qloop(j, c):
                qblock(gi, j)
                return c
            lax.fori_loop(jnp.where(gi == 0, 1, 0), NP, qloop, 0)

            @pl.when(gi == 0)
            def _():
                wo_copy().wait()

            def aloop(i, c):
                with scope('attention'):
                    attention(gi * NB0 + i)
                return c
            lax.fori_loop(0, NB0, aloop, 0)
            return carry

        lax.fori_loop(0, NGRP, group, 0)
        for cp in out_copies(B - 2, 0) + out_copies(B - 1, 1):
            cp.wait()

    def fn(x, k_cache, v_cache, wq, wo):
        return pl.pallas_call(
            kernel,
            in_specs=[pl.BlockSpec(memory_space=pl.ANY)] * 5,
            out_specs=pl.BlockSpec(memory_space=pl.ANY),
            out_shape=jax.ShapeDtypeStruct((B, SQ, D), jnp.bfloat16),
            scratch_shapes=[
                pltpu.VMEM((B, SQ, D), jnp.bfloat16),
                pltpu.VMEM((NC, D, CW), jnp.bfloat16),
                pltpu.VMEM((H * DH, D), jnp.bfloat16),
                pltpu.VMEM((2, H, SK, DH), jnp.bfloat16),
                pltpu.VMEM((2, H, SK, DH), jnp.bfloat16),
                pltpu.VMEM((NB0 * HALF, H * DH), jnp.uint32),
                pltpu.VMEM((2, SQ, D), jnp.bfloat16),
                pltpu.SemaphoreType.DMA((2, 2)),
                pltpu.SemaphoreType.DMA((NSP + 1 + SB,)),
                pltpu.SemaphoreType.DMA((PCH + 1,)),
                pltpu.SemaphoreType.DMA((1,)),
                pltpu.SemaphoreType.DMA((2, len(OUT_CUTS) - 1)),
            ],
            compiler_params=pltpu.CompilerParams(vmem_limit_bytes=120 * 1024 * 1024, disable_bounds_checks=True,
                                                 disable_semaphore_checks=True),
        )(x, k_cache, v_cache, wq, wo)
    return fn


_FN = _build()


@jax.jit
def pallas_standalone__gqa_block_cached__near_ridge_kernel(x, k_cache, v_cache, wq, wo):
    return _FN(x, k_cache, v_cache, wq, wo)
```

```python
import contextlib

import jax
import jax.numpy as jnp
from jax import lax
import jax.experimental.pallas as pl
import jax.experimental.pallas.tpu as pltpu

B, SQ, D = 16, 240, 640
H, SK, DH = 32, 1024, 128
LOG2E = 1.4426950408889634
CH = 4
CW = CH * DH
NC = H // CH
HALF = SQ // 2
LGATE = 3
NCQ = 4
RAMP = ((1, 4), (4, 3))
FILL = 16
REL_TILES = (1, 2, 3)
OUT_CUTS = (0, 512, D)


def _build(prof=False):
    qscale = (DH ** -0.5) * LOG2E
    scope = (lambda n: jax.named_scope(n)) if prof else (lambda n: contextlib.nullcontext())

    def kernel(x_hbm, k_hbm, v_hbm, wq_hbm, wo_hbm, out_hbm,
               x_v, wq_v, wo_v, kbuf, vbuf, q_v, out_v,
               kv_sem, x_sem, wq_sem, wo_sem, out_sem):
        def k_copy(b, slot):
            return pltpu.make_async_copy(k_hbm.at[b], kbuf.at[slot], kv_sem.at[0, slot])

        def v_copy(b, slot):
            return pltpu.make_async_copy(v_hbm.at[b], vbuf.at[slot], kv_sem.at[1, slot])

        pieces = []
        for nb, cnt in RAMP:
            for _ in range(cnt):
                pieces.append((sum(p[1] for p in pieces), nb))
        assert sum(p[1] for p in pieces) == B

        def x_piece(n, b0, nb):
            return pltpu.make_async_copy(x_hbm.at[pl.ds(b0, nb)], x_v.at[pl.ds(b0, nb)], x_sem.at[n])

        def wq_chunk(j, sem):
            return pltpu.make_async_copy(wq_hbm.at[:, pl.ds(j * CW, CW)], wq_v.at[j], sem)

        def wq_rest():
            return [wq_chunk(j, wq_sem.at[2]) for j in range(2, NC)]

        def wo_copy():
            return pltpu.make_async_copy(wo_hbm, wo_v, wo_sem.at[0])

        def out_copies(b, slot):
            return [pltpu.make_async_copy(out_v.at[slot, :, pl.ds(c0, c1 - c0)], out_hbm.at[b, :, pl.ds(c0, c1 - c0)],
                                          out_sem.at[slot, i])
                    for i, (c0, c1) in enumerate(zip(OUT_CUTS[:-1], OUT_CUTS[1:]))]

        def project(b0, nb, c0, nc):
            xs = x_v[pl.ds(b0, nb)].reshape(nb * SQ, D)
            w = jnp.concatenate([wq_v[c0 + t] for t in range(nc)], axis=1)
            q = jnp.dot(xs, w, preferred_element_type=jnp.float32)
            return (q * qscale).astype(jnp.bfloat16)

        def qproj(b0, nb, c):
            col = c * CW if isinstance(c, int) else pl.multiple_of(c * CW, CW)
            q_v[pl.ds(pl.multiple_of(b0 * HALF, HALF), nb * HALF), pl.ds(col, CW)] = (
                pltpu.bitcast(project(b0, nb, c, 1), jnp.uint32))

        x_piece(0, 0, pieces[0][1]).start()
        wq_chunk(0, wq_sem.at[0]).start()
        jobs = [(lambda n=n: [x_piece(n, *pieces[n])]) for n in range(1, len(pieces))]
        jobs += [lambda: [wq_chunk(1, wq_sem.at[1])], wq_rest, lambda: [k_copy(0, 0)], lambda: [v_copy(0, 0)],
                 lambda: [wo_copy()], lambda: [k_copy(1, 1)], lambda: [v_copy(1, 1)]]

        def issue(t, carry):
            for n, job in enumerate(jobs):
                @pl.when(t == n)
                def _(job=job):
                    for cp in job():
                        cp.start()
            return carry

        lax.fori_loop(0, len(jobs), issue, 0)

        def ramp_loop(n0, b0, nb, cnt):
            def body(i, carry):
                x_piece(n0 + i, b0 + i * nb, nb).wait()
                if n0 == 0:
                    @pl.when(i == 0)
                    def _():
                        wq_chunk(0, wq_sem.at[0]).wait()
                with scope('ramp%d' % nb):
                    qproj(b0 + i * nb, nb, 0)
                return carry
            lax.fori_loop(0, cnt, body, 0)

        def qblock(j, carry):
            @pl.when(j == 1)
            def _():
                wq_chunk(1, wq_sem.at[1]).wait()

            @pl.when(j == 2)
            def _():
                for cp in wq_rest():
                    cp.wait()

            with scope('qblock'):
                qproj(0, B, j)
            return carry

        n0 = b0 = 0
        for nb, cnt in RAMP:
            ramp_loop(n0, b0, nb, cnt)
            n0 += cnt
            b0 += nb * cnt
        lax.fori_loop(1, NCQ, qblock, 0)
        wo_copy().wait()

        def attention(b):
            slot = lax.bitwise_and(b, 1)

            @pl.when(b >= 2)
            def _():
                for cp in out_copies(b - 2, slot):
                    cp.wait()

            k_copy(b, slot).wait()
            v_copy(b, slot).wait()

            qall = pltpu.bitcast(q_v[pl.ds(pl.multiple_of(b * HALF, HALF), HALF), :], jnp.bfloat16)
            qall = jnp.concatenate([qall, project(b, 1, NCQ, NC - NCQ)], axis=1)
            scores, release, vgate, outs = {}, {}, {}, {}

            def qk(h):
                scores[h] = lax.dot_general(qall[:, h * DH:(h + 1) * DH], kbuf[slot, h], (((1,), (1,)), ((), ())),
                                            preferred_element_type=jnp.float32)

            def pv(h):
                sc = scores.pop(h)
                if h == H - 1:
                    zero = vgate[h - LGATE]
                    u = lax.bitcast_convert_type(sc[:, :128], jnp.uint32).reshape(SQ // 8, 8, 128)
                    w = lax.bitcast_convert_type(release[h - 1], jnp.uint32).reshape(SQ // 8, 8, 128)
                    s0 = lax.bitcast_convert_type((u | (w & zero[None])).reshape(SQ, 128), jnp.float32)
                    sc = jnp.concatenate([s0, sc[:, 128:]], axis=1)
                elif h >= 1:
                    s0 = jnp.maximum(sc[:, :128], jnp.minimum(release[h - 1], -3e38))
                    sc = jnp.concatenate([s0, sc[:, 128:]], axis=1)
                m = jnp.max(sc, axis=-1, keepdims=True)
                p = jnp.exp2(sc - m)
                tiles = [p[:, j * 128:(j + 1) * 128] for j in range(SK // 128)]
                parts = []
                for r in range(2):
                    t = tiles[r * 4:(r + 1) * 4]
                    a = (t[0] + t[1]) + (t[2] + t[3])
                    parts.append(a)
                    tiles[r * 4 + 3] = jnp.maximum(t[3], jnp.minimum(a, 0.0))
                pb = jnp.concatenate(tiles, axis=1).astype(jnp.bfloat16)
                v = vbuf[slot, h]
                if h - LGATE in vgate:
                    u = pltpu.bitcast(v, jnp.uint32)
                    u = jnp.concatenate([u[0:8] | vgate[h - LGATE], u[8:]], axis=0)
                    v = pltpu.bitcast(u, jnp.bfloat16)
                o = jnp.dot(pb, v, preferred_element_type=jnp.float32)
                release[h] = o
                l = jnp.sum(parts[0] + parts[1], axis=-1, keepdims=True)
                r = pl.reciprocal(l, approx=True)
                r = r * (2.0 - l * r)
                outs[h] = o * r
                lm = jnp.min(l.reshape(SQ // 8, 8, 1), axis=0)
                vgate[h] = jnp.broadcast_to(
                    lax.shift_right_logical(lax.bitcast_convert_type(lm, jnp.uint32), jnp.uint32(31)), (8, 128))

            def oproj(h0, h1):
                oc = jnp.concatenate([outs[t] for t in range(h0, h1)], axis=1).astype(jnp.bfloat16)
                return jnp.dot(oc, wo_v[h0 * DH:h1 * DH, :], preferred_element_type=jnp.float32)

            qk(0)
            for h in range(H - 1):
                qk(h + 1)
                pv(h)
            y = oproj(0, FILL)
            per = (SQ // 8) // len(REL_TILES)
            rel = []
            for r in range(SQ // 8):
                t, src = REL_TILES[r // per], (r % per) * len(REL_TILES)
                rel.append(y[src * 8:(src + 1) * 8, t * 128:(t + 1) * 128])
            release[H - 2] = jnp.concatenate(rel, axis=0)
            pv(H - 1)
            y = y + oproj(FILL, H)
            for cp, c0, c1 in zip(out_copies(b, slot), OUT_CUTS[:-1], OUT_CUTS[1:]):
                out_v[slot, :, c0:c1] = y[:, c0:c1].astype(out_v.dtype)
                cp.start()

            @pl.when(b + 2 < B)
            def _():
                k_copy(b + 2, slot).start()
                v_copy(b + 2, slot).start()

        def aloop(b, c):
            with scope('attention'):
                attention(b)
            return c

        lax.fori_loop(0, B, aloop, 0)
        for cp in out_copies(B - 2, 0) + out_copies(B - 1, 1):
            cp.wait()

    def fn(x, k_cache, v_cache, wq, wo):
        return pl.pallas_call(
            kernel,
            in_specs=[pl.BlockSpec(memory_space=pl.ANY)] * 5,
            out_specs=pl.BlockSpec(memory_space=pl.ANY),
            out_shape=jax.ShapeDtypeStruct((B, SQ, D), jnp.bfloat16),
            scratch_shapes=[
                pltpu.VMEM((B, SQ, D), jnp.bfloat16),
                pltpu.VMEM((NC, D, CW), jnp.bfloat16),
                pltpu.VMEM((H * DH, D), jnp.bfloat16),
                pltpu.VMEM((2, H, SK, DH), jnp.bfloat16),
                pltpu.VMEM((2, H, SK, DH), jnp.bfloat16),
                pltpu.VMEM((B * HALF, NCQ * CW), jnp.uint32),
                pltpu.VMEM((2, SQ, D), jnp.bfloat16),
                pltpu.SemaphoreType.DMA((2, 2)),
                pltpu.SemaphoreType.DMA((sum(c for _, c in RAMP),)),
                pltpu.SemaphoreType.DMA((3,)),
                pltpu.SemaphoreType.DMA((1,)),
                pltpu.SemaphoreType.DMA((2, len(OUT_CUTS) - 1)),
            ],
            compiler_params=pltpu.CompilerParams(vmem_limit_bytes=120 * 1024 * 1024, disable_bounds_checks=True,
                                                 disable_semaphore_checks=True),
        )(x, k_cache, v_cache, wq, wo)
    return fn


_FN = _build()


@jax.jit
def pallas_standalone__gqa_block_cached__near_ridge_kernel(x, k_cache, v_cache, wq, wo):
    return _FN(x, k_cache, v_cache, wq, wo)
```
